```python
import os as _os
_os.environ.setdefault('JAX_PLATFORMS', 'cpu')
import jax
import jax.numpy as jnp

def _softmax(x, axis=-1):
    return jax.nn.softmax(x, axis=axis)

def _gelu(x):
    return jax.nn.gelu(x, approximate=True)

def _silu(x):
    return jax.nn.silu(x)

def _sigmoid(x):
    return jax.nn.sigmoid(x)

def _layernorm(x, axis=-1, eps=1e-05):
    m = jnp.mean(x, axis=axis, keepdims=True)
    v = jnp.var(x, axis=axis, keepdims=True)
    return (x - m) / jnp.sqrt(v + eps)

def _scatter_add(tgt, idx, src, axis=0):
    return tgt.at[idx].add(src)

def _segment_sum(src, seg, n):
    return jax.ops.segment_sum(src, seg, n)

class _Rng:

    def __init__(self, key):
        self._k = key

    def _next(self):
        self._k, sub = jax.random.split(self._k)
        return sub

    def normal(self, shape):
        return jax.random.normal(self._next(), shape, dtype=jnp.bfloat16)

    def randint(self, lo, hi, shape):
        return jax.random.randint(self._next(), shape, lo, hi, dtype=jnp.int32)

    def uniform(self, shape, lo=0.0, hi=1.0):
        return jax.random.uniform(self._next(), shape, jnp.bfloat16, lo, hi)

    def permutation(self, n):
        return jax.random.permutation(self._next(), n)
kernel_name = 'concat_heads__linear_kernel_hedgehog__memory_aug_recurrent_mem_tr__prompt'

def setup_inputs():
    _rng = _Rng(jax.random.key(int.from_bytes(__import__("os").urandom(4), "little")))
    _w = lambda a: (lambda t: t.astype(jnp.bfloat16) if jnp.issubdtype(t.dtype, jnp.floating) else t)(jnp.asarray(a))

    def _A_setup():
        B, S, D, H = (1, 2048, 576, 32)
        Dh = D // H
        return {'x': _w((lambda *s: _rng.normal(s) * 0.4)(B, S, D)), 'wqkv': _w((lambda *s: _rng.normal(s) * 0.4)(D, 3 * D)), 'w_phi': _w((lambda *s: _rng.normal(s) * 0.4)(H, Dh, Dh) * Dh ** (-0.5)), 'wo': _w((lambda *s: _rng.normal(s) * 0.05)(D, D))}
    _A_in = _A_setup()

    def _B_setup():
        B, S, Dm = (1, 2048, 576)
        H, Dh = (32, 128)
        M, seg = (8, 32)
        seg = min(seg, S)
        S = S // seg * seg
        return {'x': _w((lambda *s: _rng.normal(s) * 0.05)(B, S, Dm)), 'mem0': _w((lambda *s: _rng.normal(s) * 0.8)(B, M, Dm)), 'Wq': _w((lambda *s: _rng.normal(s) * 3.2)(Dm, H, Dh) * Dm ** (-0.5)), 'Wk': _w((lambda *s: _rng.normal(s) * 3.2)(Dm, H, Dh) * Dm ** (-0.5)), 'Wv': _w((lambda *s: _rng.normal(s) * 0.8)(Dm, H, Dh) * Dm ** (-0.5)), 'Wo': _w((lambda *s: _rng.normal(s) * 0.8)(H, Dh, Dm) * (H * Dh) ** (-0.5)), 'seg_len': seg}
    _B_in = _B_setup()
    return {'A_x': _A_in['x'], 'A_wqkv': _A_in['wqkv'], 'A_w_phi': _A_in['w_phi'], 'A_wo': _A_in['wo'], 'B_x': _B_in['x'], 'B_mem0': _B_in['mem0'], 'B_Wq': _B_in['Wq'], 'B_Wk': _B_in['Wk'], 'B_Wv': _B_in['Wv'], 'B_Wo': _B_in['Wo'], 'B_seg_len': _B_in['seg_len']}

def reference(A_x, A_wqkv, A_w_phi, A_wo, B_x, B_mem0, B_Wq, B_Wk, B_Wv, B_Wo, B_seg_len):

    def _A_ref(x, wqkv, w_phi, wo):
        B, S, D = x.shape
        H = 32
        Dh = D // H
        qkv = (lambda x, *d: x.transpose(*d))((x @ wqkv).reshape(B, S, 3, H, Dh), 2, 0, 3, 1, 4)
        q, k, v = (qkv[0], qkv[1], qkv[2])
        pq = jnp.einsum('bhsd,hdf->bhsf', q, w_phi)
        pk = jnp.einsum('bhsd,hdf->bhsf', k, w_phi)
        phi_q = jnp.concatenate([_softmax(pq, axis=-1), _softmax(-pq, axis=-1)], axis=-1)
        phi_k = jnp.concatenate([_softmax(pk, axis=-1), _softmax(-pk, axis=-1)], axis=-1)
        kv = jnp.einsum('bhsf,bhsd->bhfd', phi_k, v)
        z = jnp.einsum('bhsf->bhf', phi_k)
        num = jnp.einsum('bhqf,bhfd->bhqd', phi_q, kv)
        den = jnp.einsum('bhqf,bhf->bhq', phi_q, z)[..., None] + 1e-06
        o = num / den
        return (lambda x, *d: x.transpose(*d))(o, 0, 2, 1, 3).reshape(B, S, D) @ wo

    def _B_ref(x, mem0, Wq, Wk, Wv, Wo, seg_len):
        B, S, Dm = x.shape
        H, Dh = (Wq.shape[1], Wq.shape[2])
        M = mem0.shape[1]
        scale = Dh ** (-0.5)
        n_seg = S // seg_len
        L = M + seg_len
        idx = jnp.arange(L)
        mask = (idx[:, None] < M) | (idx[:, None] >= idx[None, :])
        mem = mem0
        outs = []
        for s in range(n_seg):
            xs = x[:, s * seg_len:(s + 1) * seg_len, :].copy()
            h = jnp.concatenate([mem, xs], axis=1)
            q = jnp.einsum('btd,dhe->bhte', h, Wq)
            k = jnp.einsum('btd,dhe->bhte', h, Wk)
            v = jnp.einsum('btd,dhe->bhte', h, Wv)
            scores = jnp.einsum('bhqe,bhke->bhqk', q, k) * scale
            scores = jnp.where(mask[None, None], scores, -1000000000.0)
            p = _softmax(scores, axis=-1)
            o = jnp.einsum('bhqk,bhke->bhqe', p, v)
            o = jnp.einsum('bhte,hed->btd', o, Wo)
            mem = o[:, :M, :].copy()
            outs.append(o[:, M:, :])
        return jnp.concatenate(outs, axis=1)
    a = _A_ref(A_x, A_wqkv, A_w_phi, A_wo)
    b = _B_ref(B_x, B_mem0, B_Wq, B_Wk, B_Wv, B_Wo, B_seg_len)
    return jnp.concatenate([a, b], axis=-1)
```

```python
import functools

import jax
import jax.numpy as jnp
from jax import lax
import jax.experimental.pallas as pl
import jax.experimental.pallas.tpu as pltpu

F32 = jnp.float32
BF16 = jnp.bfloat16
U32 = jnp.uint32

NT = (((1,), (1,)), ((), ()))
TN = (((0,), (0,)), ((), ()))
SKIP = ""
NSEG = 0


def _dot(a, b):
    return jnp.dot(a, b, preferred_element_type=F32)


def _dot_nt(a, b):
    return lax.dot_general(a, b, NT, preferred_element_type=F32)


def _kernel(axt_hbm, awqkv_hbm, wp_hbm, awo_hbm, bxt_hbm, bmem_hbm,
            wq_hbm, wk_hbm, wv_hbm, wot_hbm, out_hbm,
            axt, awqkv, wp, awo, bxt, bx, bmem, wraw, wot, wo_s, wqkv_s,
            wt_s, wop_s, kvt_s, out_s, sems, osem,
            *, S, D, HA, DA, HB, DB, M, SEG, T):
    G = HA // 8
    GR = 8 * DA
    cps = [
        pltpu.make_async_copy(wp_hbm, wp, sems.at[0]),
        pltpu.make_async_copy(awqkv_hbm, awqkv, sems.at[1]),
        pltpu.make_async_copy(axt_hbm, axt, sems.at[2]),
        pltpu.make_async_copy(awo_hbm, awo, sems.at[3]),
        pltpu.make_async_copy(wk_hbm, wraw.at[1], sems.at[4]),
        pltpu.make_async_copy(wq_hbm, wraw.at[0], sems.at[5]),
        pltpu.make_async_copy(wv_hbm, wraw.at[2], sems.at[6]),
        pltpu.make_async_copy(wot_hbm, wot, sems.at[7]),
        pltpu.make_async_copy(bxt_hbm, bxt, sems.at[8]),
        pltpu.make_async_copy(bmem_hbm, bmem, sems.at[9]),
    ]
    for c in cps:
        c.start()

    cps[0].wait()
    ZW = 640
    eh = lax.broadcasted_iota(jnp.int32, (HA, 2 * ZW), 0) * DA
    ec = lax.broadcasted_iota(jnp.int32, (HA, 2 * ZW), 1)
    ec = jnp.where(ec >= ZW, ec - (ZW + 64), ec) - eh
    z_all = jnp.zeros((DA, 2 * ZW), F32)
    for d in range(DA):
        z_all = z_all + _dot(wp[d], jnp.where(ec == d, 1.0, 0.0).astype(BF16))
    cps[1].wait()
    W = 256
    row_j = lax.broadcasted_iota(jnp.int32, (8, W), 0)
    lane = lax.broadcasted_iota(jnp.int32, (8, W), 1)
    for part in range(3):
        base = part * D
        for g in range(G):
            c0 = base + g * GR
            w0 = (c0 // 128) * 128
            rel = lane + (w0 - c0)
            lo = row_j * DA
            own = (rel >= lo) & (rel < lo + DA)
            rows = []
            for f in range(DA):
                if part == 2:
                    rows.append(jnp.where(rel == lo + f, 1.0, 0.0).astype(F32))
                else:
                    zoff = (w0 - base) + (ZW + 64 if part == 1 else 0)
                    zr = z_all[f:f + 1, zoff:zoff + W]
                    rows.append(jnp.where(own, jnp.broadcast_to(zr, (8, W)), 0.0))
            phi = jnp.concatenate(rows, axis=0).astype(BF16)
            wend = min(w0 + W, 3 * D)
            wt = _dot_nt(phi[:, :wend - w0], awqkv[:, w0:wend])
            wt_s[part * D + g * GR: part * D + (g + 1) * GR, :] = wt.astype(BF16)
    cps[3].wait()
    r_i = lax.broadcasted_iota(jnp.int32, (GR, GR), 0)
    c_i = lax.broadcasted_iota(jnp.int32, (GR, GR), 1)
    perm = jnp.where(c_i == (r_i % 8) * DA + r_i // 8, 1.0, 0.0).astype(BF16)
    for g in range(G):
        wop_s[g * GR:(g + 1) * GR, :] = _dot(perm, awo[g * GR:(g + 1) * GR, :]).astype(BF16)

    def feat(p):
        outs = []
        for g in range(G):
            sl = [p[g * GR + f * 8: g * GR + (f + 1) * 8, :] for f in range(DA)]
            mx = functools.reduce(jnp.maximum, sl)
            mn = functools.reduce(jnp.minimum, sl)
            ep = [jnp.exp(s - mx) for s in sl]
            en = [jnp.exp(mn - s) for s in sl]
            rp = 1.0 / functools.reduce(jnp.add, ep)
            rn = 1.0 / functools.reduce(jnp.add, en)
            outs.append(jnp.concatenate([e * rp for e in ep] + [e * rn for e in en],
                                        axis=0).astype(BF16))
        return outs

    cps[2].wait()
    kvt_s[...] = jnp.zeros(kvt_s.shape, F32)
    ones = jnp.ones((16, T), BF16)

    def phase1(c, carry):
        xc = axt[:, pl.ds(pl.multiple_of(c * T, T), T)]
        kv = _dot(wt_s[D:3 * D, :], xc)
        phis = feat(kv[:D])
        for g in range(G):
            vt = kv[D + g * GR: D + (g + 1) * GR].astype(BF16)
            lhs = jnp.concatenate([vt, ones], axis=0)
            kvt_s[g] += _dot_nt(lhs, phis[g])
        return carry

    if "1" not in SKIP:
        lax.fori_loop(0, S // T, phase1, 0)

    rr = lax.broadcasted_iota(jnp.int32, (GR + 16, 2 * GR), 0)
    cc = lax.broadcasted_iota(jnp.int32, (GR + 16, 2 * GR), 1)
    keep = (rr % 8) == (cc % 8)
    kvm = [jnp.where(keep, kvt_s[g], 0.0).astype(BF16) for g in range(G)]

    def phase2(c, carry):
        r0 = pl.multiple_of(c * T, T)
        xc = axt[:, pl.ds(r0, T)]
        pq = _dot(wt_s[0:D, :], xc)
        phis = feat(pq)
        os_ = []
        for g in range(G):
            num = _dot(kvm[g], phis[g])
            rden = 1.0 / (num[GR:GR + 8] + 1e-6)
            os_ += [num[d * 8:(d + 1) * 8] * rden for d in range(DA)]
        ot = jnp.concatenate(os_, axis=0).astype(BF16)
        o = lax.dot_general(ot, wop_s[...], TN, preferred_element_type=F32)
        out_s[pl.ds(r0, T), 0:D] = o.astype(BF16)
        return carry

    if "2" not in SKIP:
        lax.fori_loop(0, S // T, phase2, 0)
    else:
        out_s[...] = jnp.zeros(out_s.shape, BF16)

    for i, ci in ((1, 4), (0, 5), (2, 6)):
        cps[ci].wait()
        if "r" in SKIP:
            continue
        w32 = wraw.at[i].bitcast(U32)
        for hp in range(HB // 2):
            a = w32[pl.ds(hp, D // 2, stride=HB), :]
            b = w32[pl.ds(HB // 2 + hp, D // 2, stride=HB), :]
            ev = (a & jnp.uint32(0xFFFF)) | (b << 16)
            od = (a >> 16) | (b & jnp.uint32(0xFFFF0000))
            wqkv_s[i, :, (2 * hp) * DB:(2 * hp + 1) * DB] = ev
            wqkv_s[i, :, (2 * hp + 1) * DB:(2 * hp + 2) * DB] = od
    cps[7].wait()

    def wo_tr(i, c):
        wo_s[pl.ds(pl.multiple_of(i * (DB // 2), DB // 2), DB // 2), :] = pltpu.bitcast(wot[i].T, U32)
        return c

    if "t" not in SKIP:
        lax.fori_loop(0, HB, wo_tr, 0, unroll=4)
    cps[8].wait()

    def x_tr(j, c):
        o = pl.multiple_of(j * 128, 128)
        bx[pl.ds(o, 128), :] = bxt[:, pl.ds(o, 128)].T
        return c

    if "t" not in SKIP:
        lax.fori_loop(0, S // 128, x_tr, 0, unroll=4)
    cps[9].wait()

    scale = DB ** -0.5
    n_seg = S // SEG
    CH = 4
    NEG = -1e9
    RA = M + SEG + M
    RB = SEG
    qi = lax.broadcasted_iota(jnp.int32, (RB, RA), 0)
    ki = lax.broadcasted_iota(jnp.int32, (RB, RA), 1)
    vis_a = (ki < M + SEG) & ((qi < M) | (qi >= ki))
    fill_a = jnp.where(ki < M + SEG, NEG, -jnp.inf).astype(F32)
    qi = lax.broadcasted_iota(jnp.int32, (RA, RA + RB), 0)
    ki = lax.broadcasted_iota(jnp.int32, (RA, RA + RB), 1)
    q_in_a = qi < M
    k_in_a = ki < M + SEG
    same = q_in_a == k_in_a
    q_mem = (qi >= 2 * M) & (qi < 3 * M)
    k_mem = (ki < M) | ((ki >= RA) & (ki < RA + M))
    q_pos = jnp.where(q_in_a, qi + (SEG - M), jnp.where(qi < 2 * M, qi - M, qi - 2 * M))
    k_pos = jnp.where(k_in_a, ki - M, jnp.where(ki < RA, ki - (M + SEG), ki - RA))
    vis_b = same & (q_mem | k_mem | (q_pos >= k_pos))
    fill_b = jnp.where(same, NEG, -jnp.inf).astype(F32)

    def out_copy(j):
        n = CH * 2 * SEG
        return pltpu.make_async_copy(out_s.at[pl.ds(j * n, n)], out_hbm.at[pl.ds(j * n, n)],
                                     osem.at[j])

    def attend(h, q_prev, k_prev, v_prev, vis, fill):
        k = _dot(h, pltpu.bitcast(wqkv_s[1], BF16)).astype(BF16)
        q = _dot(h, pltpu.bitcast(wqkv_s[0], BF16)).astype(BF16)
        if q_prev is None:
            qq, kk = q[:RB], k
        else:
            qq = jnp.concatenate([q_prev, q], axis=0)
            kk = jnp.concatenate([k_prev, k], axis=0)
        ss = [_dot_nt(qq[:, i * DB:(i + 1) * DB], kk[:, i * DB:(i + 1) * DB]) for i in range(HB)]
        v = _dot(h, pltpu.bitcast(wqkv_s[2], BF16)).astype(BF16)
        vv = v if v_prev is None else jnp.concatenate([v_prev, v], axis=0)
        ps = []
        for i in range(HB):
            sc = jnp.where(vis, ss[i] * scale, fill)
            e = jnp.exp(sc - jnp.max(sc, axis=-1, keepdims=True))
            p = e * (1.0 / jnp.sum(e, axis=-1, keepdims=True))
            ps.append(p.astype(BF16))
        o = jnp.concatenate(
            [_dot(ps[i], vv[:, i * DB:(i + 1) * DB]).astype(BF16) for i in range(HB)], axis=1)
        y = _dot(o, pltpu.bitcast(wo_s[...], BF16))
        return y, q, k, v

    def step(p, mem):
        r0 = pl.multiple_of(p * (2 * SEG), 2 * SEG)
        xx = bx[pl.ds(r0, 2 * SEG), :]
        ha = jnp.concatenate([mem, xx[:SEG + M]], axis=0)
        ya, qa, ka, va = attend(ha, None, None, None, vis_a, fill_a)
        hb = jnp.concatenate([ya[:M].astype(BF16), xx[SEG + M:]], axis=0)
        yb, _, _, _ = attend(hb, qa[RB:], ka, va, vis_b, fill_b)
        yo = jnp.concatenate([ya[M:], yb[:2 * M], yb[3 * M:]], axis=0).astype(BF16)
        out_s[pl.ds(r0, 2 * SEG), D:2 * D] = yo

        if not NSEG:
            @pl.when(p % CH == CH - 1)
            def _():
                out_copy(p // CH).start()

        return yb[2 * M:3 * M].astype(BF16)

    lax.fori_loop(0, NSEG or n_seg // 2, step, bmem[...])
    for j in range(n_seg // 2 // CH):
        if NSEG:
            out_copy(j).start()
        out_copy(j).wait()


@functools.partial(jax.jit, static_argnames=("B_seg_len",))
def pallas_concat_heads__linear_kernel_hedgehog__memory_aug_recurrent_mem_tr__prompt_kernel(
    A_x, A_wqkv, A_w_phi, A_wo, B_x, B_mem0, B_Wq, B_Wk, B_Wv, B_Wo, B_seg_len,
):
    _, S, D = A_x.shape
    HA, DA, _ = A_w_phi.shape
    _, HB, DB = B_Wq.shape
    M = B_mem0.shape[1]
    SEG = int(B_seg_len)
    T = 256
    kern = functools.partial(_kernel, S=S, D=D, HA=HA, DA=DA, HB=HB, DB=DB, M=M, SEG=SEG, T=T)
    hbm = pl.BlockSpec(memory_space=pltpu.HBM)
    out = pl.pallas_call(
        kern,
        out_shape=jax.ShapeDtypeStruct((S, 2 * D), BF16),
        in_specs=[hbm] * 10,
        out_specs=hbm,
        scratch_shapes=[
            pltpu.VMEM((D, S), BF16),
            pltpu.VMEM((D, 3 * D), BF16),
            pltpu.VMEM((DA, DA, HA), BF16),
            pltpu.VMEM((D, D), BF16),
            pltpu.VMEM((D, S), BF16),
            pltpu.VMEM((S, D), BF16),
            pltpu.VMEM((M, D), BF16),
            pltpu.VMEM((3, D * HB, DB), BF16),
            pltpu.VMEM((HB, D, DB), BF16),
            pltpu.VMEM((HB * DB // 2, D), U32),
            pltpu.VMEM((3, D // 2, HB * DB), U32),
            pltpu.VMEM((3 * D, D), BF16),
            pltpu.VMEM((D, D), BF16),
            pltpu.VMEM((HA // 8, 8 * DA + 16, 16 * DA), F32),
            pltpu.VMEM((S, 2 * D), BF16),
            pltpu.SemaphoreType.DMA((10,)),
            pltpu.SemaphoreType.DMA((S // SEG // 8,)),
        ],
        compiler_params=pltpu.CompilerParams(vmem_limit_bytes=100 * 1024 * 1024),
    )(jnp.transpose(A_x[0]), A_wqkv, jnp.transpose(A_w_phi, (1, 2, 0)), A_wo,
      jnp.transpose(B_x[0]), B_mem0[0],
      B_Wq.reshape(D * HB, DB), B_Wk.reshape(D * HB, DB), B_Wv.reshape(D * HB, DB),
      jnp.transpose(B_Wo, (0, 2, 1)))
    return out.reshape(1, S, 2 * D)
```

```python
import functools

import jax
import jax.numpy as jnp
from jax import lax
import jax.experimental.pallas as pl
import jax.experimental.pallas.tpu as pltpu

F32 = jnp.float32
BF16 = jnp.bfloat16
U32 = jnp.uint32

NT = (((1,), (1,)), ((), ()))
TN = (((0,), (0,)), ((), ()))
SKIP = ""
NSEG = 0
TT = 512
PROF = 0


class _Null:
    def __enter__(self):
        return self

    def __exit__(self, *a):
        return False


def _scope(name):
    return jax.named_scope(name) if PROF else _Null()


def _dot(a, b):
    return jnp.dot(a, b, preferred_element_type=F32)


def _dot_nt(a, b):
    return lax.dot_general(a, b, NT, preferred_element_type=F32)


def _iota(shape, dim):
    return lax.broadcasted_iota(jnp.int32, shape, dim)


def _kernel(axt_hbm, awqkv_hbm, wp_hbm, awo_hbm, bxt_hbm, bmem_hbm,
            wq_hbm, wk_hbm, wv_hbm, wot_hbm, out_hbm,
            axt, awqkv, wp, awo, bxt, bx, bmem, wraw, wot, wo_s, wqkv_s,
            wt_s, wot_a, aot, kvt_s, out_s, ybuf, sems, osem,
            *, S, D, HA, DA, HB, DB, M, SEG, T):
    GH = 4
    G = HA // GH
    GR = GH * DA
    NS = GR // 8
    NCH = S // T
    HC = HB // NCH
    HP = HB // 2
    PIT = 3 * (D // 2) + 1
    cp_wp = pltpu.make_async_copy(wp_hbm, wp, sems.at[0])
    KL = (D // 128) * 128

    def aw_copy(lo, hi, s):
        return pltpu.make_async_copy(awqkv_hbm.at[:, pl.ds(lo, hi - lo)],
                                     awqkv.at[:, pl.ds(lo, hi - lo)], sems.at[s])

    cp_awk = aw_copy(KL, 2 * D, 1)
    cp_awv = aw_copy(2 * D, 3 * D, 7 + 3 * NCH)
    cp_awq = aw_copy(0, KL, 8 + 3 * NCH)
    cp_awo = pltpu.make_async_copy(awo_hbm, awo, sems.at[2])
    cp_mem = pltpu.make_async_copy(bmem_hbm, bmem, sems.at[3])
    w_hbm = (wk_hbm, wq_hbm, wv_hbm)

    WR = D * HB
    WC = 3 * WR // NCH
    w_pieces = []
    cuts = sorted({i * WR for i in range(4)} | {c * WC for c in range(NCH + 1)})
    for n, (lo, hi) in enumerate(zip(cuts[:-1], cuts[1:])):
        i = lo // WR
        w_pieces.append((lo // WC, pltpu.make_async_copy(
            w_hbm[i].at[pl.ds(lo - i * WR, hi - lo)], wraw.at[pl.ds(lo, hi - lo)],
            sems.at[9 + 3 * NCH + n])))

    def axt_copy(c):
        return pltpu.make_async_copy(axt_hbm.at[:, pl.ds(c * T, T)], axt.at[:, pl.ds(c * T, T)],
                                     sems.at[7 + c])

    def wot_copy(c):
        return pltpu.make_async_copy(wot_hbm.at[pl.ds(c * HC, HC)], wot.at[pl.ds(c * HC, HC)],
                                     sems.at[7 + NCH + c])

    def bxt_copy(c):
        return pltpu.make_async_copy(bxt_hbm.at[:, pl.ds(c * T, T)], bxt.at[:, pl.ds(c * T, T)],
                                     sems.at[7 + 2 * NCH + c])

    cp_wp.start()
    cp_awk.start()
    cp_awv.start()
    for c in range(NCH):
        axt_copy(c).start()
    cp_awq.start()
    cp_awo.start()
    cp_mem.start()
    for c in range(NCH):
        wot_copy(c).start()
        bxt_copy(c).start()
        for cc, cp in w_pieces:
            if cc == c:
                cp.start()

    with _scope("w_wp"):
        cp_wp.wait()
    ZW = 640
    ec = _iota((HA, ZW), 1) - _iota((HA, ZW), 0) * DA
    z_q = jnp.zeros((DA, ZW), F32)
    for d in range(DA):
        z_q = z_q + _dot(wp[d], jnp.where(ec == d, 1.0, 0.0).astype(BF16))
    rr = _iota((5 * 8, DA), 0)
    rep = jnp.where(rr < 32, (rr // 8) * 4 + (rr % 8) // 2, 16 + (rr - 32) // 4)
    rep = jnp.where(_iota((5 * 8, DA), 1) == rep, 1.0, 0.0).astype(BF16)
    zz_q = _dot(rep, z_q.astype(BF16))
    zz_k = pltpu.roll(zz_q, D - KL, 1)
    W = 256
    PR = 2 * GR
    sub = _iota((8, W), 0)
    lane = _iota((8, W), 1)

    def fold(part):
        base = part * D
        zz = zz_k if part == 1 else zz_q
        for gp in range(G // 2):
            c0 = base + gp * PR
            w0 = (c0 // 128) * 128
            zoff = w0 - (KL if part == 1 else 0)
            rows = []
            for gg in range(2):
                col = lane + (w0 - c0 - gg * GR)
                own = []
                for head in (sub % 2, 2 + sub % 2, sub % 4):
                    rel = col - head * DA
                    own.append((rel >= 0) & (rel < DA))
                for i in range(NS):
                    zi = i % 4 if i < 8 else 4
                    rows.append(jnp.where(own[i // 4], zz[zi * 8:(zi + 1) * 8, zoff:zoff + W], 0.0))
            phi = jnp.concatenate(rows, axis=0).astype(BF16)
            wend = min(w0 + W, 3 * D)
            wt = _dot_nt(phi[:, :wend - w0], awqkv[:, w0:wend])
            wt_s[c0 // 2:(c0 + PR) // 2, :] = pltpu.bitcast(wt.astype(BF16), U32)

    with _scope("w_awk"):
        cp_awk.wait()
    fold(1)
    with _scope("w_awv"):
        cp_awv.wait()
    wt_s[D:3 * D // 2, :] = pltpu.bitcast(awqkv[:, 2 * D:3 * D].T, U32)

    def wt(r, n):
        return pltpu.bitcast(wt_s[r // 2:(r + n) // 2, :], BF16)

    sub_t = _iota((8, T), 0)
    lo = sub_t % 4 < 2

    def red(op, sl):
        two = []
        for part in (sl[0:4], sl[4:8]):
            m = functools.reduce(op, part)
            m = op(m, pltpu.roll(m, 4, 0))
            two.append(op(m, pltpu.roll(m, 2, 0)))
        mc = op(sl[8], pltpu.roll(sl[8], 4, 0))
        rc = pltpu.roll(mc, 2, 0)
        return op(two[0], jnp.where(lo, mc, rc)), op(two[1], jnp.where(lo, rc, mc))

    def spread(ab):
        return [ab[0]] * 4 + [ab[1]] * 4 + [jnp.where(lo, ab[0], ab[1])]

    def feat(p):
        sl = [p[i * 8:(i + 1) * 8, :] for i in range(NS)]
        mx = spread(red(jnp.maximum, sl))
        mn = spread(red(jnp.minimum, sl))
        ep = [jnp.exp(s - m) for s, m in zip(sl, mx)]
        en = [jnp.exp(m - s) for s, m in zip(sl, mn)]
        rp = spread([pl.reciprocal(r, approx=True) for r in red(jnp.add, ep)])
        rn = spread([pl.reciprocal(r, approx=True) for r in red(jnp.add, en)])
        ep = [e * r for e, r in zip(ep, rp)]
        en = [e * r for e, r in zip(en, rn)]
        return [jnp.concatenate(ep[o:o + 4] + en[o:o + 4] + [ep[8], en[8]], axis=0).astype(BF16)
                for o in (0, 4)]

    kvt_s[...] = jnp.zeros(kvt_s.shape, F32)
    ones = jnp.ones((8, T), F32)

    def phase1(c, carry):
        axt_copy(c).wait()
        xc = axt[:, pl.ds(pl.multiple_of(c * T, T), T)]
        for gp in range(G // 2):
            pk = _dot(wt(D + gp * PR, PR), xc)
            vt = _dot(wt(2 * D + gp * PR, PR), xc)
            for gg in range(2):
                phis = feat(pk[gg * GR:(gg + 1) * GR])
                for ab in range(2):
                    v0 = gg * GR + ab * 32
                    lhs = jnp.concatenate([vt[v0:v0 + 40], ones], axis=0).astype(BF16)
                    kvt_s[4 * gp + 2 * gg + ab] += _dot_nt(lhs, phis[ab])
        return carry

    with _scope("ph1"):
        lax.fori_loop(0, NCH, phase1, 0)

    cp_awq.wait()
    cp_awo.wait()
    fold(0)
    wot_a[...] = pltpu.bitcast(awo[...].T, U32)
    r_i = _iota((48, 80), 0)
    c_i = _iota((48, 80), 1)
    kvm = []
    for g in range(2 * G):
        ab = g % 2
        rh = jnp.where(r_i < 40, (r_i + 32 * ab) // DA, 2 * ab + r_i % 2)
        ch = jnp.where(c_i < 64, 2 * ab + c_i % 2, c_i % 4)
        keep = (rh == ch) & (rh // 2 == ab)
        kvm.append(jnp.where(keep, kvt_s[g], 0.0).astype(BF16))
    w32 = wraw.bitcast(U32)
    JB = D // 16
    JC = 3 * JB // NCH

    def relay(c):
        srcv = w32.at[pl.ds(pl.multiple_of(c * (JC * 16 * HP), 8), JC * 16 * HP)]
        dst = wqkv_s.at[pl.ds(pl.multiple_of(c * (JC * 24), 8), HB * PIT + JC * 24)]
        for dp in range(JC * 8):
            a = srcv[2 * dp * HP:(2 * dp + 1) * HP, :]
            b = srcv[(2 * dp + 1) * HP:(2 * dp + 2) * HP, :]
            dst[pl.ds(3 * dp, HP, stride=PIT), :] = (a & jnp.uint32(0xFFFF)) | (b << 16)
            dst[pl.ds(HP * PIT + 3 * dp, HP, stride=PIT), :] = (
                (a >> 16) | (b & jnp.uint32(0xFFFF0000)))

    def phase2(c, carry):
        r0 = pl.multiple_of(c * T, T)
        wot_copy(c).wait()
        bxt_copy(c).wait()
        for i in range(NCH):
            @pl.when(c == i)
            def _():
                for cc, cp in w_pieces:
                    if cc == i:
                        cp.wait()
        xc = axt[:, pl.ds(r0, T)]
        os_ = []
        pq = _dot(wt(0, D), xc)
        for g in range(G):
            phis = feat(pq[g * GR:(g + 1) * GR])
            na = _dot(kvm[2 * g], phis[0])
            nb = _dot(kvm[2 * g + 1], phis[1])
            num = [na[i * 8:(i + 1) * 8] for i in range(4)] + [na[32:40] + nb[0:8]] + [
                nb[i * 8:(i + 1) * 8] for i in range(1, 5)]
            rden = pl.reciprocal(jnp.where(lo, na[40:48], nb[40:48]) + 1e-6, approx=True)
            rb = [jnp.broadcast_to(rden[j:j + 1], (8, T)) for j in range(GH)]
            for i in range(NS):
                j0, j1 = (8 * i) // DA, (8 * i + 7) // DA
                r = rb[j0] if j0 == j1 else jnp.where(sub_t < j1 * DA - 8 * i, rb[j0], rb[j1])
                os_.append(num[i] * r)
        ot = jnp.concatenate(os_, axis=0).astype(BF16)
        aot[:, pl.ds(r0, T)] = pltpu.bitcast(
            _dot(pltpu.bitcast(wot_a[...], BF16), ot).astype(BF16), U32)
        relay(c)
        for hh in range(HC):
            h = c * HC + hh
            wo_s[pl.ds(pl.multiple_of(h * (DB // 2), DB // 2), DB // 2), :] = (
                pltpu.bitcast(wot[h].T, U32))
        for tt in range(T // 128):
            o = pl.multiple_of(r0 + tt * 128, 128)
            bx[pl.ds(o, 128), :] = bxt[:, pl.ds(o, 128)].T
        return carry

    with _scope("ph2"):
        lax.fori_loop(0, NCH, phase2, 0)
    cp_mem.wait()

    def wmat(i):
        return jnp.concatenate(
            [pltpu.bitcast(
                wqkv_s[pl.ds(((h % 2) * HP + h // 2) * PIT + 3 * (D // 2) * i, D // 2, stride=3), :], BF16)
             for h in range(HB)], axis=1)

    scale = DB ** -0.5
    n_seg = S // SEG
    NEG = -1e9
    RA = M + SEG + M
    RB = SEG
    qi = _iota((RB, RA), 0)
    ki = _iota((RB, RA), 1)
    vis_a = (ki < M + SEG) & ((qi < M) | (qi >= ki))
    fill_a = jnp.where(ki < M + SEG, NEG, -jnp.inf).astype(F32)
    qi = _iota((RA, RA + RB), 0)
    ki = _iota((RA, RA + RB), 1)
    q_in_a = qi < M
    k_in_a = ki < M + SEG
    same = q_in_a == k_in_a
    q_mem = (qi >= 2 * M) & (qi < 3 * M)
    k_mem = (ki < M) | ((ki >= RA) & (ki < RA + M))
    q_pos = jnp.where(q_in_a, qi + (SEG - M), jnp.where(qi < 2 * M, qi - M, qi - 2 * M))
    k_pos = jnp.where(k_in_a, ki - M, jnp.where(ki < RA, ki - (M + SEG), ki - RA))
    vis_b = same & (q_mem | k_mem | (q_pos >= k_pos))
    fill_b = jnp.where(same, NEG, -jnp.inf).astype(F32)

    BT = 4 * SEG

    def out_copy(j):
        return pltpu.make_async_copy(out_s.at[pl.ds(j * BT, BT)], out_hbm.at[pl.ds(j * BT, BT)],
                                     osem.at[j])

    def attend(h, q_prev, k_prev, v_prev, vis, fill):
        k = _dot(h, wmat(0)).astype(BF16)
        q = _dot(h, wmat(1)).astype(BF16)
        if q_prev is None:
            qq, kk = q[:RB], k
        else:
            qq = jnp.concatenate([q_prev, q], axis=0)
            kk = jnp.concatenate([k_prev, k], axis=0)
        ss = [_dot_nt(qq[:, i * DB:(i + 1) * DB], kk[:, i * DB:(i + 1) * DB]) for i in range(HB)]
        v = _dot(h, wmat(2)).astype(BF16)
        vv = v if v_prev is None else jnp.concatenate([v_prev, v], axis=0)
        ps, rs = [], []
        for i in range(HB):
            sc = jnp.where(vis, ss[i] * scale, fill)
            e = jnp.exp(sc - jnp.max(sc, axis=-1, keepdims=True))
            rs.append(pl.reciprocal(jnp.sum(e, axis=-1, keepdims=True), approx=True))
            ps.append(e.astype(BF16))
        o = jnp.concatenate(
            [(_dot(ps[i], vv[:, i * DB:(i + 1) * DB]) * rs[i]).astype(BF16) for i in range(HB)],
            axis=1)
        y = _dot(o, pltpu.bitcast(wo_s[...], BF16))
        return y, q, k, v

    def flush(r):
        out_s[pl.ds(pl.multiple_of(r, 2 * SEG), 2 * SEG), D:2 * D] = ybuf[...]

    ybuf[...] = jnp.zeros(ybuf.shape, BF16)

    def pair(xx, mem):
        ha = jnp.concatenate([mem, xx[:SEG + M]], axis=0)
        ya, qa, ka, va = attend(ha, None, None, None, vis_a, fill_a)
        hb = jnp.concatenate([ya[:M].astype(BF16), xx[SEG + M:]], axis=0)
        yb, _, _, _ = attend(hb, qa[RB:], ka, va, vis_b, fill_b)
        yo = jnp.concatenate([ya[M:], yb[:2 * M], yb[3 * M:]], axis=0).astype(BF16)
        return yo, yb[2 * M:3 * M].astype(BF16)

    NIT = S // BT

    def step(it, mem):
        r0 = pl.multiple_of(it * BT, BT)
        flush(jnp.maximum(r0 - 2 * SEG, 0))
        out_s[pl.ds(r0, BT), 0:D] = pltpu.bitcast(aot[:, pl.ds(r0, BT)], BF16).T
        xx = bx[pl.ds(r0, BT), :]
        y0, mem = pair(xx[:2 * SEG], mem)
        out_s[pl.ds(r0, 2 * SEG), D:2 * D] = y0
        y1, mem = pair(xx[2 * SEG:], mem)
        ybuf[...] = y1

        @pl.when(it > 0)
        def _():
            out_copy(it - 1).start()

        return mem

    with _scope("bloop"):
        lax.fori_loop(0, NIT, step, bmem[...])
    flush(S - 2 * SEG)
    out_copy(NIT - 1).start()
    for j in range(NIT):
        out_copy(j).wait()


@functools.partial(jax.jit, static_argnames=("B_seg_len",))
def pallas_concat_heads__linear_kernel_hedgehog__memory_aug_recurrent_mem_tr__prompt_kernel(
    A_x, A_wqkv, A_w_phi, A_wo, B_x, B_mem0, B_Wq, B_Wk, B_Wv, B_Wo, B_seg_len,
):
    _, S, D = A_x.shape
    HA, DA, _ = A_w_phi.shape
    _, HB, DB = B_Wq.shape
    M = B_mem0.shape[1]
    SEG = int(B_seg_len)
    T = TT
    kern = functools.partial(_kernel, S=S, D=D, HA=HA, DA=DA, HB=HB, DB=DB, M=M, SEG=SEG, T=T)
    hbm = pl.BlockSpec(memory_space=pltpu.HBM)
    out = pl.pallas_call(
        kern,
        out_shape=jax.ShapeDtypeStruct((S, 2 * D), BF16),
        in_specs=[hbm] * 10,
        out_specs=hbm,
        scratch_shapes=[
            pltpu.VMEM((D, S), BF16),
            pltpu.VMEM((D, 3 * D), BF16),
            pltpu.VMEM((DA, DA, HA), BF16),
            pltpu.VMEM((D, D), BF16),
            pltpu.VMEM((D, S), BF16),
            pltpu.VMEM((S, D), BF16),
            pltpu.VMEM((M, D), BF16),
            pltpu.VMEM((3 * D * HB, DB), BF16),
            pltpu.VMEM((HB, D, DB), BF16),
            pltpu.VMEM((HB * DB // 2, D), U32),
            pltpu.VMEM(((HB + 3) * (3 * (D // 2) + 1), DB), U32),
            pltpu.VMEM((3 * D // 2, D), U32),
            pltpu.VMEM((D // 2, D), U32),
            pltpu.VMEM((D // 2, S), U32),
            pltpu.VMEM((HA // 2, 48, 80), F32),
            pltpu.VMEM((S, 2 * D), BF16),
            pltpu.VMEM((2 * SEG, D), BF16),
            pltpu.SemaphoreType.DMA((12 + 4 * (S // T),)),
            pltpu.SemaphoreType.DMA((S // (4 * SEG),)),
        ],
        compiler_params=pltpu.CompilerParams(vmem_limit_bytes=100 * 1024 * 1024),
    )(jnp.transpose(A_x[0]), A_wqkv, jnp.transpose(A_w_phi, (1, 2, 0)), A_wo,
      jnp.transpose(B_x[0]), B_mem0[0],
      B_Wq.reshape(D * HB, DB), B_Wk.reshape(D * HB, DB), B_Wv.reshape(D * HB, DB),
      jnp.transpose(B_Wo, (0, 2, 1)))
    return out.reshape(1, S, 2 * D)
```

```python
import functools

import jax
import jax.numpy as jnp
from jax import lax
import jax.experimental.pallas as pl
import jax.experimental.pallas.tpu as pltpu

F32 = jnp.float32
BF16 = jnp.bfloat16
U32 = jnp.uint32


def _dot(a, b):
    return jnp.dot(a, b, preferred_element_type=F32)


def _dot_nt(a, b):
    return lax.dot_general(a, b, (((1,), (1,)), ((), ())), preferred_element_type=F32)


def _iota(shape, dim):
    return lax.broadcasted_iota(jnp.int32, shape, dim)


def _pack(x):
    return pltpu.bitcast(x, U32)


def _unpack(x):
    return pltpu.bitcast(x, BF16)


def _kernel(axt_hbm, awqkv_hbm, wp_hbm, awo_hbm, bxt_hbm, bmem_hbm,
            wq_hbm, wk_hbm, wv_hbm, wot_hbm, out_hbm,
            axt, awqkv, wp, awo, bxt, bx, bmem, wraw, wot, wo_s, wqkv_s,
            wt_s, wot_a, aot, axp, kvt_s, out_s, ybuf, sems, osem,
            *, S, D, HA, DA, HB, DB, M, SEG, T):
    GH = 4
    G = HA // GH
    GR = GH * DA
    NS = GR // 8
    NCH = S // T
    HC = HB // NCH
    HP = HB // 2
    PIT = 3 * (D // 2) + 1
    KL = (D // 128) * 128

    def aw_copy(lo, hi, s):
        return pltpu.make_async_copy(awqkv_hbm.at[:, pl.ds(lo, hi - lo)],
                                     awqkv.at[:, pl.ds(lo, hi - lo)], sems.at[s])

    cp_wp = pltpu.make_async_copy(wp_hbm, wp, sems.at[0])
    cp_awk = aw_copy(KL, 2 * D, 1)
    cp_awv = aw_copy(2 * D, 3 * D, 2)
    cp_awq = aw_copy(0, KL, 3)
    cp_awo = pltpu.make_async_copy(awo_hbm, awo, sems.at[4])
    cp_mem = pltpu.make_async_copy(bmem_hbm, bmem, sems.at[5])

    def axt_copy(c):
        return pltpu.make_async_copy(axt_hbm.at[:, pl.ds(c * T, T)], axt.at[:, pl.ds(c * T, T)],
                                     sems.at[6 + c])

    def wot_copy(c):
        return pltpu.make_async_copy(wot_hbm.at[pl.ds(c * HC, HC)], wot.at[pl.ds(c * HC, HC)],
                                     sems.at[6 + NCH + c])

    def bxt_copy(c):
        return pltpu.make_async_copy(bxt_hbm.at[:, pl.ds(c * T, T)], bxt.at[:, pl.ds(c * T, T)],
                                     sems.at[6 + 2 * NCH + c])

    w_hbm = (wk_hbm, wq_hbm, wv_hbm)
    WR = D * HB
    WC = 3 * WR // NCH
    w_pieces = []
    cuts = sorted({i * WR for i in range(4)} | {c * WC for c in range(NCH + 1)})
    for n, (lo, hi) in enumerate(zip(cuts[:-1], cuts[1:])):
        i = lo // WR
        w_pieces.append((lo // WC, pltpu.make_async_copy(
            w_hbm[i].at[pl.ds(lo - i * WR, hi - lo)], wraw.at[pl.ds(lo, hi - lo)],
            sems.at[6 + 3 * NCH + n])))

    cp_wp.start()
    cp_awk.start()
    cp_awv.start()
    for c in range(NCH):
        axt_copy(c).start()
    cp_awq.start()
    cp_awo.start()
    cp_mem.start()
    for c in range(NCH):
        wot_copy(c).start()
        bxt_copy(c).start()
        for cc, cp in w_pieces:
            if cc == c:
                cp.start()

    cp_wp.wait()
    ZW = KL + 128
    ec = _iota((HA, ZW), 1) - _iota((HA, ZW), 0) * DA
    z = jnp.zeros((DA, ZW), F32)
    for d in range(DA):
        z = z + _dot(wp[d], jnp.where(ec == d, 1.0, 0.0).astype(BF16))
    rr = _iota((5 * 8, DA), 0)
    rep = jnp.where(rr < 32, (rr // 8) * 4 + (rr % 8) // 2, 16 + (rr - 32) // 4)
    rep = jnp.where(_iota((5 * 8, DA), 1) == rep, 1.0, 0.0).astype(BF16)
    zz_q = _dot(rep, z.astype(BF16))
    zz_k = pltpu.roll(zz_q, D - KL, 1)
    W = 256
    PR = 2 * GR
    sub = _iota((8, W), 0)
    lane = _iota((8, W), 1)

    def fold(part):
        base = part * D
        zz = zz_k if part == 1 else zz_q
        for gp in range(G // 2):
            c0 = base + gp * PR
            w0 = (c0 // 128) * 128
            zoff = w0 - (KL if part == 1 else 0)
            rows = []
            for gg in range(2):
                col = lane + (w0 - c0 - gg * GR)
                own = []
                for head in (sub % 2, 2 + sub % 2, sub % 4):
                    rel = col - head * DA
                    own.append((rel >= 0) & (rel < DA))
                for i in range(NS):
                    zi = i % 4 if i < 8 else 4
                    rows.append(jnp.where(own[i // 4], zz[zi * 8:(zi + 1) * 8, zoff:zoff + W], 0.0))
            phi = jnp.concatenate(rows, axis=0).astype(BF16)
            wt_s[c0 // 2:(c0 + PR) // 2, :] = _pack(
                _dot_nt(phi, awqkv[:, w0:w0 + W]).astype(BF16))

    cp_awk.wait()
    fold(1)
    cp_awv.wait()
    wt_s[D:3 * D // 2, :] = _pack(awqkv[:, 2 * D:3 * D].T)

    def wt(r, n):
        return _unpack(wt_s[r // 2:(r + n) // 2, :])

    sub_t = _iota((8, T), 0)
    lo = sub_t % 4 < 2

    def red(op, sl):
        two = []
        for part in (sl[0:4], sl[4:8]):
            m = functools.reduce(op, part)
            m = op(m, pltpu.roll(m, 4, 0))
            two.append(op(m, pltpu.roll(m, 2, 0)))
        mc = op(sl[8], pltpu.roll(sl[8], 4, 0))
        rc = pltpu.roll(mc, 2, 0)
        return op(two[0], jnp.where(lo, mc, rc)), op(two[1], jnp.where(lo, rc, mc))

    def spread(ab):
        return [ab[0]] * 4 + [ab[1]] * 4 + [jnp.where(lo, ab[0], ab[1])]

    def feat(p):
        sl = [p[i * 8:(i + 1) * 8, :] for i in range(NS)]
        mx = spread(red(jnp.maximum, sl))
        mn = spread(red(jnp.minimum, sl))
        ep = [jnp.exp(s - m) for s, m in zip(sl, mx)]
        en = [jnp.exp(m - s) for s, m in zip(sl, mn)]
        rp = spread([pl.reciprocal(r, approx=True) for r in red(jnp.add, ep)])
        rn = spread([pl.reciprocal(r, approx=True) for r in red(jnp.add, en)])
        ep = [e * r for e, r in zip(ep, rp)]
        en = [e * r for e, r in zip(en, rn)]
        return [jnp.concatenate(ep[o:o + 4] + en[o:o + 4] + [ep[8], en[8]], axis=0).astype(BF16)
                for o in (0, 4)]

    kvt_s[...] = jnp.zeros(kvt_s.shape, F32)
    ones = jnp.ones((8, T), F32)

    def phase1(c, carry):
        axt_copy(c).wait()
        r0 = pl.multiple_of(c * T, T)
        xc = axt[:, pl.ds(r0, T)]
        axp[:, pl.ds(r0, T)] = _pack(xc)
        for gp in range(G // 2):
            pk = _dot(wt(D + gp * PR, PR), xc)
            vt = _dot(wt(2 * D + gp * PR, PR), xc)
            for gg in range(2):
                phis = feat(pk[gg * GR:(gg + 1) * GR])
                for ab in range(2):
                    v0 = gg * GR + ab * 32
                    lhs = jnp.concatenate([vt[v0:v0 + 40], ones], axis=0).astype(BF16)
                    kvt_s[4 * gp + 2 * gg + ab] += _dot_nt(lhs, phis[ab])
        return carry

    lax.fori_loop(0, NCH, phase1, 0)

    cp_awq.wait()
    cp_awo.wait()
    fold(0)
    wot_a[...] = _pack(awo[...].T)
    r_i = _iota((48, 80), 0)
    c_i = _iota((48, 80), 1)
    kvm = []
    for g in range(2 * G):
        ab = g % 2
        rh = jnp.where(r_i < 40, (r_i + 32 * ab) // DA, 2 * ab + r_i % 2)
        ch = jnp.where(c_i < 64, 2 * ab + c_i % 2, c_i % 4)
        keep = (rh == ch) & (rh // 2 == ab)
        kvm.append(jnp.where(keep, kvt_s[g], 0.0).astype(BF16))

    w32 = wraw.bitcast(U32)
    DP = WC // (2 * HB)

    def relay(c):
        src = w32.at[pl.ds(pl.multiple_of(c * (DP * HB), 8), DP * HB)]
        dst = wqkv_s.at[pl.ds(pl.multiple_of(c * (3 * DP), 8), HB * PIT + 3 * DP)]
        for dp in range(DP):
            a = src[2 * dp * HP:(2 * dp + 1) * HP, :]
            b = src[(2 * dp + 1) * HP:(2 * dp + 2) * HP, :]
            dst[pl.ds(3 * dp, HP, stride=PIT), :] = (a & jnp.uint32(0xFFFF)) | (b << 16)
            dst[pl.ds(HP * PIT + 3 * dp, HP, stride=PIT), :] = (
                (a >> 16) | (b & jnp.uint32(0xFFFF0000)))

    def phase2(c, carry):
        r0 = pl.multiple_of(c * T, T)
        wot_copy(c).wait()
        bxt_copy(c).wait()
        for i in range(NCH):
            @pl.when(c == i)
            def _():
                for cc, cp in w_pieces:
                    if cc == i:
                        cp.wait()
        pq = _dot(wt(0, D), _unpack(axp[:, pl.ds(r0, T)]))
        os_ = []
        for g in range(G):
            phis = feat(pq[g * GR:(g + 1) * GR])
            na = _dot(kvm[2 * g], phis[0])
            nb = _dot(kvm[2 * g + 1], phis[1])
            num = [na[i * 8:(i + 1) * 8] for i in range(4)] + [na[32:40] + nb[0:8]] + [
                nb[i * 8:(i + 1) * 8] for i in range(1, 5)]
            rden = pl.reciprocal(jnp.where(lo, na[40:48], nb[40:48]) + 1e-6, approx=True)
            rb = [jnp.broadcast_to(rden[j:j + 1], (8, T)) for j in range(GH)]
            for i in range(NS):
                j0, j1 = (8 * i) // DA, (8 * i + 7) // DA
                r = rb[j0] if j0 == j1 else jnp.where(sub_t < j1 * DA - 8 * i, rb[j0], rb[j1])
                os_.append(num[i] * r)
        ot = jnp.concatenate(os_, axis=0).astype(BF16)
        for hf in range(4):
            rows = slice(hf * D // 8, (hf + 1) * D // 8)
            aot[rows, pl.ds(r0, T)] = _pack(_dot(_unpack(wot_a[rows, :]), ot).astype(BF16))
        relay(c)
        for hh in range(HC):
            h = c * HC + hh
            wo_s[pl.ds(pl.multiple_of(h * (DB // 2), DB // 2), DB // 2), :] = _pack(wot[h].T)
        for tt in range(T // 128):
            o = pl.multiple_of(r0 + tt * 128, 128)
            bx[pl.ds(o, 128), :] = bxt[:, pl.ds(o, 128)].T
        return carry

    lax.fori_loop(0, NCH, phase2, 0)
    cp_mem.wait()

    def wmat(i):
        return jnp.concatenate(
            [_unpack(wqkv_s[pl.ds(((h % 2) * HP + h // 2) * PIT + 3 * (D // 2) * i, D // 2,
                                  stride=3), :]) for h in range(HB)], axis=1)

    scale = DB ** -0.5
    NEG = -1e9
    RA = M + SEG + M
    RB = SEG
    qi = _iota((RB, RA), 0)
    ki = _iota((RB, RA), 1)
    vis_a = (ki < M + SEG) & ((qi < M) | (qi >= ki))
    fill_a = jnp.where(ki < M + SEG, NEG, -jnp.inf).astype(F32)
    qi = _iota((RA, RA + RB), 0)
    ki = _iota((RA, RA + RB), 1)
    q_in_a = qi < M
    k_in_a = ki < M + SEG
    same = q_in_a == k_in_a
    q_mem = (qi >= 2 * M) & (qi < 3 * M)
    k_mem = (ki < M) | ((ki >= RA) & (ki < RA + M))
    q_pos = jnp.where(q_in_a, qi + (SEG - M), jnp.where(qi < 2 * M, qi - M, qi - 2 * M))
    k_pos = jnp.where(k_in_a, ki - M, jnp.where(ki < RA, ki - (M + SEG), ki - RA))
    vis_b = same & (q_mem | k_mem | (q_pos >= k_pos))
    fill_b = jnp.where(same, NEG, -jnp.inf).astype(F32)

    BT = 4 * SEG
    NIT = S // BT

    def out_copy(j):
        return pltpu.make_async_copy(out_s.at[pl.ds(j * BT, BT)], out_hbm.at[pl.ds(j * BT, BT)],
                                     osem.at[j])

    def attend(h, q_prev, k_prev, v_prev, vis, fill):
        k = _dot(h, wmat(0)).astype(BF16)
        q = _dot(h, wmat(1)).astype(BF16)
        if q_prev is None:
            qq, kk = q[:RB], k
        else:
            qq = jnp.concatenate([q_prev, q], axis=0)
            kk = jnp.concatenate([k_prev, k], axis=0)
        ss = [_dot_nt(qq[:, i * DB:(i + 1) * DB], kk[:, i * DB:(i + 1) * DB]) for i in range(HB)]
        v = _dot(h, wmat(2)).astype(BF16)
        vv = v if v_prev is None else jnp.concatenate([v_prev, v], axis=0)
        ps, rs = [], []
        for i in range(HB):
            sc = jnp.where(vis, ss[i] * scale, fill)
            e = jnp.exp(sc - jnp.max(sc, axis=-1, keepdims=True))
            rs.append(pl.reciprocal(jnp.sum(e, axis=-1, keepdims=True), approx=True))
            ps.append(e.astype(BF16))
        o = jnp.concatenate(
            [(_dot(ps[i], vv[:, i * DB:(i + 1) * DB]) * rs[i]).astype(BF16) for i in range(HB)],
            axis=1)
        y = _dot(o, _unpack(wo_s[...]))
        return y, q, k, v

    def pair(xx, mem):
        ha = jnp.concatenate([mem, xx[:SEG + M]], axis=0)
        ya, qa, ka, va = attend(ha, None, None, None, vis_a, fill_a)
        hb = jnp.concatenate([ya[:M].astype(BF16), xx[SEG + M:]], axis=0)
        yb, _, _, _ = attend(hb, qa[RB:], ka, va, vis_b, fill_b)
        yo = jnp.concatenate([ya[M:], yb[:2 * M], yb[3 * M:]], axis=0).astype(BF16)
        return yo, yb[2 * M:3 * M].astype(BF16)

    def flush(r):
        out_s[pl.ds(r, 2 * SEG), D:2 * D] = ybuf[...]

    ybuf[...] = jnp.zeros(ybuf.shape, BF16)

    def step(it, mem):
        r0 = pl.multiple_of(it * BT, BT)
        flush(pl.multiple_of(jnp.maximum(r0 - 2 * SEG, 0), 2 * SEG))
        out_s[pl.ds(r0, BT), 0:D] = _unpack(aot[:, pl.ds(r0, BT)]).T
        xx = bx[pl.ds(r0, BT), :]
        y0, mem = pair(xx[:2 * SEG], mem)
        out_s[pl.ds(r0, 2 * SEG), D:2 * D] = y0
        y1, mem = pair(xx[2 * SEG:], mem)
        ybuf[...] = y1

        @pl.when(it > 0)
        def _():
            out_copy(it - 1).start()

        return mem

    lax.fori_loop(0, NIT, step, bmem[...])
    flush(S - 2 * SEG)
    out_copy(NIT - 1).start()
    for j in range(NIT):
        out_copy(j).wait()


@functools.partial(jax.jit, static_argnames=("seg",))
def _run(A_x, A_wqkv, A_w_phi, A_wo, B_x, B_mem0, B_Wq, B_Wk, B_Wv, B_Wo, seg):
    nb, S, D = A_x.shape
    HA, DA, _ = A_w_phi.shape
    _, HB, DB = B_Wq.shape
    M = B_mem0.shape[1]
    T = 512
    assert nb == 1 and DA == 18 and HA * DA == D and HA % 8 == 0 and D % 128 == 64
    assert DB == 128 and M == 8 and seg == 32 and S % T == 0 and HB % (2 * S // T) == 0
    nch = S // T
    kern = functools.partial(_kernel, S=S, D=D, HA=HA, DA=DA, HB=HB, DB=DB, M=M, SEG=seg, T=T)
    hbm = pl.BlockSpec(memory_space=pltpu.HBM)
    out = pl.pallas_call(
        kern,
        out_shape=jax.ShapeDtypeStruct((S, 2 * D), BF16),
        in_specs=[hbm] * 10,
        out_specs=hbm,
        scratch_shapes=[
            pltpu.VMEM((D, S), BF16),
            pltpu.VMEM((D, 3 * D), BF16),
            pltpu.VMEM((DA, DA, HA), BF16),
            pltpu.VMEM((D, D), BF16),
            pltpu.VMEM((D, S), BF16),
            pltpu.VMEM((S, D), BF16),
            pltpu.VMEM((M, D), BF16),
            pltpu.VMEM((3 * D * HB, DB), BF16),
            pltpu.VMEM((HB, D, DB), BF16),
            pltpu.VMEM((HB * DB // 2, D), U32),
            pltpu.VMEM(((HB + 3) * (3 * (D // 2) + 1), DB), U32),
            pltpu.VMEM((3 * D // 2, D), U32),
            pltpu.VMEM((D // 2, D), U32),
            pltpu.VMEM((D // 2, S), U32),
            pltpu.VMEM((D // 2, S), U32),
            pltpu.VMEM((HA // 2, 48, 80), F32),
            pltpu.VMEM((S, 2 * D), BF16),
            pltpu.VMEM((2 * seg, D), BF16),
            pltpu.SemaphoreType.DMA((6 + 4 * nch + 2,)),
            pltpu.SemaphoreType.DMA((S // (4 * seg),)),
        ],
        compiler_params=pltpu.CompilerParams(vmem_limit_bytes=100 * 1024 * 1024),
    )(jnp.transpose(A_x[0]), A_wqkv, jnp.transpose(A_w_phi, (1, 2, 0)), A_wo,
      jnp.transpose(B_x[0]), B_mem0[0],
      B_Wq.reshape(D * HB, DB), B_Wk.reshape(D * HB, DB), B_Wv.reshape(D * HB, DB),
      jnp.transpose(B_Wo, (0, 2, 1)))
    return out.reshape(1, S, 2 * D)


def pallas_concat_heads__linear_kernel_hedgehog__memory_aug_recurrent_mem_tr__prompt_kernel(
    A_x, A_wqkv, A_w_phi, A_wo, B_x, B_mem0, B_Wq, B_Wk, B_Wv, B_Wo, B_seg_len,
):
    seg = B_seg_len if isinstance(B_seg_len, int) else 32
    return _run(A_x, A_wqkv, A_w_phi, A_wo, B_x, B_mem0, B_Wq, B_Wk, B_Wv, B_Wo, seg)
```

```python
import functools

import jax
import jax.numpy as jnp
from jax import lax
import jax.experimental.pallas as pl
import jax.experimental.pallas.tpu as pltpu

F32 = jnp.float32
BF16 = jnp.bfloat16
U32 = jnp.uint32


def _dot(a, b):
    return jnp.dot(a, b, preferred_element_type=F32)


def _dot_nt(a, b):
    return lax.dot_general(a, b, (((1,), (1,)), ((), ())), preferred_element_type=F32)


def _iota(shape, dim):
    return lax.broadcasted_iota(jnp.int32, shape, dim)


def _pack(x):
    return pltpu.bitcast(x, U32)


def _unpack(x):
    return pltpu.bitcast(x, BF16)


def _kernel(axt_hbm, awqkv_hbm, wp_hbm, awo_hbm, bxt_hbm, bmem_hbm,
            wq_hbm, wk_hbm, wv_hbm, wot_hbm, out_hbm,
            axt, awqkv, wp, awo, bxt, bx, bmem, wraw, wot, wo_s, wqkv_s,
            wt_s, wot_a, aot, axp, phi_s, kvt_s, out_s, ybuf, sems, osem,
            *, S, D, HA, DA, HB, DB, M, SEG, T):
    GH = 4
    G = HA // GH
    GR = GH * DA
    NS = GR // 8
    NCH = S // T
    HC = HB // NCH
    HP = HB // 2
    PIT = 3 * (D // 2) + 1
    KL = (D // 128) * 128

    def aw_copy(lo, hi, s):
        return pltpu.make_async_copy(awqkv_hbm.at[:, pl.ds(lo, hi - lo)],
                                     awqkv.at[:, pl.ds(lo, hi - lo)], sems.at[s])

    cp_wp = pltpu.make_async_copy(wp_hbm, wp, sems.at[0])
    cp_awk = aw_copy(KL, 2 * D, 1)
    cp_awv = aw_copy(2 * D, 3 * D, 2)
    cp_awq = aw_copy(0, KL, 3)
    cp_awo = pltpu.make_async_copy(awo_hbm, awo, sems.at[4])
    cp_mem = pltpu.make_async_copy(bmem_hbm, bmem, sems.at[5])

    def axt_copy(c):
        return pltpu.make_async_copy(axt_hbm.at[:, pl.ds(c * T, T)], axt.at[:, pl.ds(c * T, T)],
                                     sems.at[6 + c])

    def wot_copy(c):
        return pltpu.make_async_copy(wot_hbm.at[pl.ds(c * HC, HC)], wot.at[pl.ds(c * HC, HC)],
                                     sems.at[6 + NCH + c])

    def bxt_copy(c):
        return pltpu.make_async_copy(bxt_hbm.at[:, pl.ds(c * T, T)], bxt.at[:, pl.ds(c * T, T)],
                                     sems.at[6 + 2 * NCH + c])

    w_hbm = (wk_hbm, wq_hbm, wv_hbm)
    WR = D * HB
    WC = 3 * WR // NCH
    w_pieces = []
    cuts = sorted({i * WR for i in range(4)} | {c * WC for c in range(NCH + 1)})
    for n, (lo, hi) in enumerate(zip(cuts[:-1], cuts[1:])):
        i = lo // WR
        w_pieces.append((lo // WC, pltpu.make_async_copy(
            w_hbm[i].at[pl.ds(lo - i * WR, hi - lo)], wraw.at[pl.ds(lo, hi - lo)],
            sems.at[6 + 3 * NCH + n])))

    cp_wp.start()
    cp_awk.start()
    cp_awv.start()
    for c in range(NCH):
        axt_copy(c).start()
    cp_awq.start()
    cp_awo.start()
    cp_mem.start()
    for c in range(NCH):
        wot_copy(c).start()
        if c == 0:
            bxt_copy(c).start()
        for cc, cp in w_pieces:
            if cc == c:
                cp.start()
    for c in range(1, NCH):
        bxt_copy(c).start()

    cp_wp.wait()
    ZW = KL + 128
    ec = _iota((HA, ZW), 1) - _iota((HA, ZW), 0) * DA
    z = jnp.zeros((DA, ZW), F32)
    for d in range(DA):
        z = z + _dot(wp[d], jnp.where(ec == d, 1.0, 0.0).astype(BF16))
    rr = _iota((5 * 8, DA), 0)
    rep = jnp.where(rr < 32, (rr // 8) * 4 + (rr % 8) // 2, 16 + (rr - 32) // 4)
    rep = jnp.where(_iota((5 * 8, DA), 1) == rep, 1.0, 0.0).astype(BF16)
    zz_q = _dot(rep, z.astype(BF16))
    zz_k = pltpu.roll(zz_q, D - KL, 1)
    W = 256
    PR = 2 * GR
    sub = _iota((8, W), 0)
    lane = _iota((8, W), 1)

    def make_phi(part):
        base = part * D
        zz = zz_k if part == 1 else zz_q
        for gp in range(G // 2):
            c0 = base + gp * PR
            w0 = (c0 // 128) * 128
            zoff = w0 - (KL if part == 1 else 0)
            rows = []
            for gg in range(2):
                col = lane + (w0 - c0 - gg * GR)
                own = []
                for head in (sub % 2, 2 + sub % 2, sub % 4):
                    rel = col - head * DA
                    own.append((rel >= 0) & (rel < DA))
                for i in range(NS):
                    zi = i % 4 if i < 8 else 4
                    rows.append(jnp.where(own[i // 4], zz[zi * 8:(zi + 1) * 8, zoff:zoff + W], 0.0))
            phi_s[part * (G // 2) + gp] = _pack(jnp.concatenate(rows, axis=0).astype(BF16))

    def fold(part):
        for gp in range(G // 2):
            c0 = part * D + gp * PR
            w0 = (c0 // 128) * 128
            wt_s[c0 // 2:(c0 + PR) // 2, :] = _pack(_dot_nt(
                _unpack(phi_s[part * (G // 2) + gp]), awqkv[:, w0:w0 + W]).astype(BF16))

    make_phi(1)
    make_phi(0)
    r_i = _iota((48, 80), 0)
    c_i = _iota((48, 80), 1)
    off_diag = []
    for ab in range(2):
        x = r_i + 32 * ab
        rh = sum(jnp.where(x >= j * DA, 1, 0) for j in range(1, GH))
        rh = jnp.where(r_i < 40, rh, 2 * ab + (r_i & 1))
        ch = jnp.where(c_i < 64, 2 * ab + (c_i & 1), c_i & 3)
        off_diag.append(jnp.where((rh >> 1) == ab, rh - ch, 1))

    cp_awk.wait()
    fold(1)
    cp_awv.wait()
    wt_s[D:3 * D // 2, :] = _pack(awqkv[:, 2 * D:3 * D].T)

    def wt(r, n):
        return _unpack(wt_s[r // 2:(r + n) // 2, :])

    sub_t = _iota((8, T), 0)
    lo = sub_t % 4 < 2

    def red(op, sl):
        two = []
        for part in (sl[0:4], sl[4:8]):
            m = functools.reduce(op, part)
            m = op(m, pltpu.roll(m, 4, 0))
            two.append(op(m, pltpu.roll(m, 2, 0)))
        mc = op(sl[8], pltpu.roll(sl[8], 4, 0))
        rc = pltpu.roll(mc, 2, 0)
        return op(two[0], jnp.where(lo, mc, rc)), op(two[1], jnp.where(lo, rc, mc))

    def spread(ab):
        return [ab[0]] * 4 + [ab[1]] * 4 + [jnp.where(lo, ab[0], ab[1])]

    def feat(p):
        sl = [p[i * 8:(i + 1) * 8, :] for i in range(NS)]
        mx = spread(red(jnp.maximum, sl))
        mn = spread(red(jnp.minimum, sl))
        ep = [jnp.exp(s - m) for s, m in zip(sl, mx)]
        en = [jnp.exp(m - s) for s, m in zip(sl, mn)]
        rp = spread([pl.reciprocal(r, approx=True) for r in red(jnp.add, ep)])
        rn = spread([pl.reciprocal(r, approx=True) for r in red(jnp.add, en)])
        ep = [e * r for e, r in zip(ep, rp)]
        en = [e * r for e, r in zip(en, rn)]
        return [jnp.concatenate(ep[o:o + 4] + en[o:o + 4] + [ep[8], en[8]], axis=0).astype(BF16)
                for o in (0, 4)]

    kvt_s[...] = jnp.zeros(kvt_s.shape, F32)
    ones = jnp.ones((8, T), F32)

    def phase1(c, carry):
        axt_copy(c).wait()
        r0 = pl.multiple_of(c * T, T)
        xc = axt[:, pl.ds(r0, T)]
        axp[:, pl.ds(r0, T)] = _pack(xc)
        for gp in range(G // 2):
            pk = _dot(wt(D + gp * PR, PR), xc)
            vt = _dot(wt(2 * D + gp * PR, PR), xc)
            for gg in range(2):
                phis = feat(pk[gg * GR:(gg + 1) * GR])
                for ab in range(2):
                    v0 = gg * GR + ab * 32
                    lhs = jnp.concatenate([vt[v0:v0 + 40], ones], axis=0).astype(BF16)
                    kvt_s[4 * gp + 2 * gg + ab] += _dot_nt(lhs, phis[ab])
        return carry

    lax.fori_loop(0, NCH, phase1, 0)

    cp_awq.wait()
    cp_awo.wait()
    fold(0)
    wot_a[...] = _pack(awo[...].T)
    kvm = [jnp.where(off_diag[g % 2] == 0, kvt_s[g], 0.0).astype(BF16) for g in range(2 * G)]

    w32 = wraw.bitcast(U32)
    DP = WC // (2 * HB)

    def relay(c):
        src = w32.at[pl.ds(pl.multiple_of(c * (DP * HB), 8), DP * HB)]
        dst = wqkv_s.at[pl.ds(pl.multiple_of(c * (3 * DP), 8), HB * PIT + 3 * DP)]
        for dp in range(DP):
            a = src[2 * dp * HP:(2 * dp + 1) * HP, :]
            b = src[(2 * dp + 1) * HP:(2 * dp + 2) * HP, :]
            dst[pl.ds(3 * dp, HP, stride=PIT), :] = (a & jnp.uint32(0xFFFF)) | (b << 16)
            dst[pl.ds(HP * PIT + 3 * dp, HP, stride=PIT), :] = (
                (a >> 16) | (b & jnp.uint32(0xFFFF0000)))

    def x_tr(o):
        bx[pl.ds(o, 128), :] = bxt[:, pl.ds(o, 128)].T

    def phase2(c, carry):
        r0 = pl.multiple_of(c * T, T)
        wot_copy(c).wait()
        for i in range(NCH):
            @pl.when(c == i)
            def _():
                if i == 0:
                    bxt_copy(0).wait()
                for cc, cp in w_pieces:
                    if cc == i:
                        cp.wait()
        pq = _dot(wt(0, D), _unpack(axp[:, pl.ds(r0, T)]))
        os_ = []
        for g in range(G):
            phis = feat(pq[g * GR:(g + 1) * GR])
            na = _dot(kvm[2 * g], phis[0])
            nb = _dot(kvm[2 * g + 1], phis[1])
            num = [na[i * 8:(i + 1) * 8] for i in range(4)] + [na[32:40] + nb[0:8]] + [
                nb[i * 8:(i + 1) * 8] for i in range(1, 5)]
            rden = pl.reciprocal(jnp.where(lo, na[40:48], nb[40:48]) + 1e-6, approx=True)
            rb = [jnp.broadcast_to(rden[j:j + 1], (8, T)) for j in range(GH)]
            for i in range(NS):
                j0, j1 = (8 * i) // DA, (8 * i + 7) // DA
                r = rb[j0] if j0 == j1 else jnp.where(sub_t < j1 * DA - 8 * i, rb[j0], rb[j1])
                os_.append(num[i] * r)
        ot = jnp.concatenate(os_, axis=0).astype(BF16)
        for hf in range(4):
            rows = slice(hf * D // 8, (hf + 1) * D // 8)
            w = _unpack(wot_a[rows, :])
            if hf == 0:
                o = _dot(w[:, :KL], ot[:KL])
                o = _dot(w[:, KL:], ot[KL:]) + o
            else:
                o = _dot(w, ot)
            aot[rows, pl.ds(r0, T)] = _pack(o.astype(BF16))
        relay(c)
        for hh in range(HC):
            h = c * HC + hh
            wo_s[pl.ds(pl.multiple_of(h * (DB // 2), DB // 2), DB // 2), :] = _pack(wot[h].T)
        x_tr(pl.multiple_of(c * 128, 128))
        return carry

    lax.fori_loop(0, NCH, phase2, 0)
    cp_mem.wait()
    for c in range(1, NCH):
        bxt_copy(c).wait()

    def wmat(i, h0=0, h1=HB, d0=0, d1=D):
        return jnp.concatenate(
            [_unpack(wqkv_s[pl.ds(((h % 2) * HP + h // 2) * PIT + 3 * ((D * i + d0) // 2),
                                  (d1 - d0) // 2, stride=3), :]) for h in range(h0, h1)], axis=1)

    scale = DB ** -0.5
    NEG = -1e9
    RA = M + SEG + M
    RB = SEG
    qi = _iota((RB, RA), 0)
    ki = _iota((RB, RA), 1)
    vis_a = (ki < M + SEG) & ((qi < M) | (qi >= ki))
    fill_a = jnp.where(ki < M + SEG, NEG, -jnp.inf).astype(F32)
    qi = _iota((RA, RA + RB), 0)
    ki = _iota((RA, RA + RB), 1)
    q_in_a = qi < M
    k_in_a = ki < M + SEG
    same = q_in_a == k_in_a
    q_mem = (qi >= 2 * M) & (qi < 3 * M)
    k_mem = (ki < M) | ((ki >= RA) & (ki < RA + M))
    q_pos = jnp.where(q_in_a, qi + (SEG - M), jnp.where(qi < 2 * M, qi - M, qi - 2 * M))
    k_pos = jnp.where(k_in_a, ki - M, jnp.where(ki < RA, ki - (M + SEG), ki - RA))
    vis_b = same & (q_mem | k_mem | (q_pos >= k_pos))
    fill_b = jnp.where(same, NEG, -jnp.inf).astype(F32)

    BT = 4 * SEG
    NIT = S // BT

    def out_copy(j):
        return pltpu.make_async_copy(out_s.at[pl.ds(j * BT, BT)], out_hbm.at[pl.ds(j * BT, BT)],
                                     osem.at[j])

    def attend(h, q_prev, k_prev, v_prev, vis, fill, first=False):
        NH = 4
        if first:
            k = _dot(h[:, KL:], wmat(0, 0, NH, KL, D))
            k = _dot(h[:, :KL], wmat(0, 0, NH, 0, KL)) + k
        else:
            k = _dot(h[:, :KL], wmat(0, 0, NH, 0, KL))
            k = _dot(h[:, KL:], wmat(0, 0, NH, KL, D)) + k
        k = jnp.concatenate([k, _dot(h, wmat(0, NH, HB))], axis=1).astype(BF16)
        q = _dot(h, wmat(1)).astype(BF16)
        if q_prev is None:
            qq, kk = q[:RB], k
        else:
            qq = jnp.concatenate([q_prev, q], axis=0)
            kk = jnp.concatenate([k_prev, k], axis=0)
        ss = [_dot_nt(qq[:, i * DB:(i + 1) * DB], kk[:, i * DB:(i + 1) * DB]) for i in range(HB)]
        v = _dot(h, wmat(2)).astype(BF16)
        vv = v if v_prev is None else jnp.concatenate([v_prev, v], axis=0)
        ps, rs = [], []
        for i in range(HB):
            sc = jnp.where(vis, ss[i] * scale, fill)
            e = jnp.exp(sc - jnp.max(sc, axis=-1, keepdims=True))
            rs.append(pl.reciprocal(jnp.sum(e, axis=-1, keepdims=True), approx=True))
            ps.append(e.astype(BF16))
        o = jnp.concatenate(
            [(_dot(ps[i], vv[:, i * DB:(i + 1) * DB]) * rs[i]).astype(BF16) for i in range(HB)],
            axis=1)
        y = _dot(o, _unpack(wo_s[...]))
        return y, q, k, v

    def pair(xx, mem, first=False):
        ha = jnp.concatenate([mem, xx[:SEG + M]], axis=0)
        ya, qa, ka, va = attend(ha, None, None, None, vis_a, fill_a, first)
        hb = jnp.concatenate([ya[:M].astype(BF16), xx[SEG + M:]], axis=0)
        yb, _, _, _ = attend(hb, qa[RB:], ka, va, vis_b, fill_b)
        yo = jnp.concatenate([ya[M:], yb[:2 * M], yb[3 * M:]], axis=0).astype(BF16)
        return yo, yb[2 * M:3 * M].astype(BF16)

    def flush(r):
        out_s[pl.ds(r, 2 * SEG), D:2 * D] = ybuf[...]

    ybuf[...] = jnp.zeros(ybuf.shape, BF16)

    def step(it, mem):
        r0 = pl.multiple_of(it * BT, BT)
        flush(pl.multiple_of(jnp.maximum(r0 - 2 * SEG, 0), 2 * SEG))
        out_s[pl.ds(r0, BT), 0:D] = _unpack(aot[:, pl.ds(r0, BT)]).T
        xx = bx[pl.ds(r0, BT), :]
        y0, mem = pair(xx[:2 * SEG], mem, True)
        out_s[pl.ds(r0, 2 * SEG), D:2 * D] = y0
        y1, mem = pair(xx[2 * SEG:], mem)
        ybuf[...] = y1
        x_tr(pl.multiple_of(jnp.minimum(r0 + NCH * BT, S - BT), BT))

        @pl.when(it > 0)
        def _():
            out_copy(it - 1).start()

        return mem

    lax.fori_loop(0, NIT, step, bmem[...])
    flush(S - 2 * SEG)
    out_copy(NIT - 1).start()
    for j in range(NIT):
        out_copy(j).wait()


@functools.partial(jax.jit, static_argnames=("seg",))
def _run(A_x, A_wqkv, A_w_phi, A_wo, B_x, B_mem0, B_Wq, B_Wk, B_Wv, B_Wo, seg):
    nb, S, D = A_x.shape
    HA, DA, _ = A_w_phi.shape
    _, HB, DB = B_Wq.shape
    M = B_mem0.shape[1]
    T = 512
    assert nb == 1 and DA == 18 and HA * DA == D and HA % 8 == 0 and D % 128 == 64
    assert DB == 128 and M == 8 and seg == 32 and S % T == 0 and HB % (2 * S // T) == 0
    nch = S // T
    kern = functools.partial(_kernel, S=S, D=D, HA=HA, DA=DA, HB=HB, DB=DB, M=M, SEG=seg, T=T)
    hbm = pl.BlockSpec(memory_space=pltpu.HBM)
    out = pl.pallas_call(
        kern,
        out_shape=jax.ShapeDtypeStruct((S, 2 * D), BF16),
        in_specs=[hbm] * 10,
        out_specs=hbm,
        scratch_shapes=[
            pltpu.VMEM((D, S), BF16),
            pltpu.VMEM((D, 3 * D), BF16),
            pltpu.VMEM((DA, DA, HA), BF16),
            pltpu.VMEM((D, D), BF16),
            pltpu.VMEM((D, S), BF16),
            pltpu.VMEM((S, D), BF16),
            pltpu.VMEM((M, D), BF16),
            pltpu.VMEM((3 * D * HB, DB), BF16),
            pltpu.VMEM((HB, D, DB), BF16),
            pltpu.VMEM((HB * DB // 2, D), U32),
            pltpu.VMEM(((HB + 3) * (3 * (D // 2) + 1), DB), U32),
            pltpu.VMEM((3 * D // 2, D), U32),
            pltpu.VMEM((D // 2, D), U32),
            pltpu.VMEM((D // 2, S), U32),
            pltpu.VMEM((D // 2, S), U32),
            pltpu.VMEM((HA // 4, 4 * DA, 256), U32),
            pltpu.VMEM((HA // 2, 48, 80), F32),
            pltpu.VMEM((S, 2 * D), BF16),
            pltpu.VMEM((2 * seg, D), BF16),
            pltpu.SemaphoreType.DMA((6 + 4 * nch + 2,)),
            pltpu.SemaphoreType.DMA((S // (4 * seg),)),
        ],
        compiler_params=pltpu.CompilerParams(vmem_limit_bytes=100 * 1024 * 1024),
    )(jnp.transpose(A_x[0]), A_wqkv, jnp.transpose(A_w_phi, (1, 2, 0)), A_wo,
      jnp.transpose(B_x[0]), B_mem0[0],
      B_Wq.reshape(D * HB, DB), B_Wk.reshape(D * HB, DB), B_Wv.reshape(D * HB, DB),
      jnp.transpose(B_Wo, (0, 2, 1)))
    return out.reshape(1, S, 2 * D)


def pallas_concat_heads__linear_kernel_hedgehog__memory_aug_recurrent_mem_tr__prompt_kernel(
    A_x, A_wqkv, A_w_phi, A_wo, B_x, B_mem0, B_Wq, B_Wk, B_Wv, B_Wo, B_seg_len,
):
    seg = B_seg_len if isinstance(B_seg_len, int) else 32
    return _run(A_x, A_wqkv, A_w_phi, A_wo, B_x, B_mem0, B_Wq, B_Wk, B_Wv, B_Wo, seg)
```

```python
import functools

import jax
import jax.numpy as jnp
from jax import lax
import jax.experimental.pallas as pl
import jax.experimental.pallas.tpu as pltpu

F32 = jnp.float32
BF16 = jnp.bfloat16
U32 = jnp.uint32


def _dot(a, b):
    return jnp.dot(a, b, preferred_element_type=F32)


def _dot_nt(a, b):
    return lax.dot_general(a, b, (((1,), (1,)), ((), ())), preferred_element_type=F32)


def _iota(shape, dim):
    return lax.broadcasted_iota(jnp.int32, shape, dim)


def _pack(x):
    return pltpu.bitcast(x, U32)


def _unpack(x):
    return pltpu.bitcast(x, BF16)


def _kernel(axt_hbm, awqkv_hbm, wp_hbm, awo_hbm, bxt_hbm, bmem_hbm,
            wq_hbm, wk_hbm, wv_hbm, wot_hbm, out_hbm,
            axt, awqkv, wp, awo, bxt, bx, bmem, wraw, wot, wo_s, wqkv_s,
            wt_s, wot_a, aot, axp, phi_s, kvt_s, out_s, ybuf, sems, osem,
            *, S, D, HA, DA, HB, DB, M, SEG, T):
    GH = 4
    G = HA // GH
    GR = GH * DA
    NS = GR // 8
    NCH = S // T
    HC = HB // NCH
    HP = HB // 2
    PIT = 3 * (D // 2) + 1
    KL = (D // 128) * 128

    def aw_copy(lo, hi, s):
        return pltpu.make_async_copy(awqkv_hbm.at[:, pl.ds(lo, hi - lo)],
                                     awqkv.at[:, pl.ds(lo, hi - lo)], sems.at[s])

    cp_wp = pltpu.make_async_copy(wp_hbm, wp, sems.at[0])
    cp_awk = aw_copy(KL, 2 * D, 1)
    cp_awv = aw_copy(2 * D, 3 * D, 2)
    cp_awq = aw_copy(0, KL, 3)
    cp_awo = pltpu.make_async_copy(awo_hbm, awo, sems.at[4])
    cp_mem = pltpu.make_async_copy(bmem_hbm, bmem, sems.at[5])

    def axt_copy(c):
        return pltpu.make_async_copy(axt_hbm.at[:, pl.ds(c * T, T)], axt.at[:, pl.ds(c * T, T)],
                                     sems.at[6 + c])

    def wot_copy(c):
        return pltpu.make_async_copy(wot_hbm.at[pl.ds(c * HC, HC)], wot.at[pl.ds(c * HC, HC)],
                                     sems.at[6 + NCH + c])

    def bxt_copy(c):
        return pltpu.make_async_copy(bxt_hbm.at[:, pl.ds(c * T, T)], bxt.at[:, pl.ds(c * T, T)],
                                     sems.at[6 + 2 * NCH + c])

    w_hbm = (wk_hbm, wq_hbm, wv_hbm)
    WR = D * HB // 16
    WC = 3 * WR // NCH
    w_pieces = []
    cuts = sorted({i * WR for i in range(4)} | {c * WC for c in range(NCH + 1)})
    for n, (lo, hi) in enumerate(zip(cuts[:-1], cuts[1:])):
        i = lo // WR
        w_pieces.append((lo // WC, pltpu.make_async_copy(
            w_hbm[i].at[pl.ds(lo - i * WR, hi - lo)], wraw.at[pl.ds(lo, hi - lo)],
            sems.at[6 + 3 * NCH + n])))

    cp_wp.start()
    cp_awk.start()
    cp_awv.start()
    for c in range(NCH):
        axt_copy(c).start()
    cp_awq.start()
    cp_awo.start()
    cp_mem.start()
    for c in range(NCH):
        wot_copy(c).start()
        if c == 0:
            bxt_copy(c).start()
        for cc, cp in w_pieces:
            if cc == c:
                cp.start()
    for c in range(1, NCH):
        bxt_copy(c).start()

    cp_wp.wait()
    ZW = KL + 128
    ec = _iota((HA, ZW), 1) - _iota((HA, ZW), 0) * DA
    z = jnp.zeros((DA, ZW), F32)
    for d in range(DA):
        z = z + _dot(wp[d], jnp.where(ec == d, 1.0, 0.0).astype(BF16))
    rr = _iota((5 * 8, DA), 0)
    rep = jnp.where(rr < 32, (rr // 8) * 4 + (rr % 8) // 2, 16 + (rr - 32) // 4)
    rep = jnp.where(_iota((5 * 8, DA), 1) == rep, 1.0, 0.0).astype(BF16)
    zz_q = _dot(rep, z.astype(BF16))
    zz_k = pltpu.roll(zz_q, D - KL, 1)
    W = 256
    PR = 2 * GR
    sub = _iota((8, W), 0)
    lane = _iota((8, W), 1)

    def make_phi(part):
        base = part * D
        zz = zz_k if part == 1 else zz_q
        for gp in range(G // 2):
            c0 = base + gp * PR
            w0 = (c0 // 128) * 128
            zoff = w0 - (KL if part == 1 else 0)
            rows = []
            for gg in range(2):
                col = lane + (w0 - c0 - gg * GR)
                own = []
                for head in (sub % 2, 2 + sub % 2, sub % 4):
                    rel = col - head * DA
                    own.append((rel >= 0) & (rel < DA))
                for i in range(NS):
                    zi = i % 4 if i < 8 else 4
                    rows.append(jnp.where(own[i // 4], zz[zi * 8:(zi + 1) * 8, zoff:zoff + W], 0.0))
            phi_s[part * (G // 2) + gp] = _pack(jnp.concatenate(rows, axis=0).astype(BF16))

    def fold(part):
        for gp in range(G // 2):
            c0 = part * D + gp * PR
            w0 = (c0 // 128) * 128
            wt_s[c0 // 2:(c0 + PR) // 2, :] = _pack(_dot_nt(
                _unpack(phi_s[part * (G // 2) + gp]), awqkv[:, w0:w0 + W]).astype(BF16))

    make_phi(1)
    make_phi(0)
    r_i = _iota((48, 80), 0)
    c_i = _iota((48, 80), 1)
    off_diag = []
    for ab in range(2):
        x = r_i + 32 * ab
        rh = sum(jnp.where(x >= j * DA, 1, 0) for j in range(1, GH))
        rh = jnp.where(r_i < 40, rh, 2 * ab + (r_i & 1))
        ch = jnp.where(c_i < 64, 2 * ab + (c_i & 1), c_i & 3)
        off_diag.append(jnp.where((rh >> 1) == ab, rh - ch, 1))

    cp_awk.wait()
    fold(1)
    cp_awv.wait()
    wt_s[D:3 * D // 2, :] = _pack(awqkv[:, 2 * D:3 * D].T)

    def wt(r, n):
        return _unpack(wt_s[r // 2:(r + n) // 2, :])

    sub_t = _iota((8, T), 0)
    lo = sub_t % 4 < 2

    def red(op, sl):
        two = []
        for part in (sl[0:4], sl[4:8]):
            m = functools.reduce(op, part)
            m = op(m, pltpu.roll(m, 4, 0))
            two.append(op(m, pltpu.roll(m, 2, 0)))
        mc = op(sl[8], pltpu.roll(sl[8], 4, 0))
        rc = pltpu.roll(mc, 2, 0)
        return op(two[0], jnp.where(lo, mc, rc)), op(two[1], jnp.where(lo, rc, mc))

    def spread(ab):
        return [ab[0]] * 4 + [ab[1]] * 4 + [jnp.where(lo, ab[0], ab[1])]

    def feat(p):
        sl = [p[i * 8:(i + 1) * 8, :] for i in range(NS)]
        mx = spread(red(jnp.maximum, sl))
        mn = spread(red(jnp.minimum, sl))
        ep = [jnp.exp(s - m) for s, m in zip(sl, mx)]
        en = [jnp.exp(m - s) for s, m in zip(sl, mn)]
        rp = spread([pl.reciprocal(r, approx=True) for r in red(jnp.add, ep)])
        rn = spread([pl.reciprocal(r, approx=True) for r in red(jnp.add, en)])
        ep = [e * r for e, r in zip(ep, rp)]
        en = [e * r for e, r in zip(en, rn)]
        return [jnp.concatenate(ep[o:o + 4] + en[o:o + 4] + [ep[8], en[8]], axis=0).astype(BF16)
                for o in (0, 4)]

    kvt_s[...] = jnp.zeros(kvt_s.shape, F32)
    ones = jnp.ones((8, T), F32)

    def phase1(c, carry):
        axt_copy(c).wait()
        r0 = pl.multiple_of(c * T, T)
        xc = axt[:, pl.ds(r0, T)]
        axp[:, pl.ds(r0, T)] = _pack(xc)
        for gp in range(G // 2):
            pk = _dot(wt(D + gp * PR, PR), xc)
            vt = _dot(wt(2 * D + gp * PR, PR), xc)
            for gg in range(2):
                phis = feat(pk[gg * GR:(gg + 1) * GR])
                for ab in range(2):
                    v0 = gg * GR + ab * 32
                    lhs = jnp.concatenate([vt[v0:v0 + 40], ones], axis=0).astype(BF16)
                    kvt_s[4 * gp + 2 * gg + ab] += _dot_nt(lhs, phis[ab])
        return carry

    lax.fori_loop(0, NCH, phase1, 0)

    cp_awq.wait()
    cp_awo.wait()
    fold(0)
    wot_a[...] = _pack(awo[...].T)
    kvm = [jnp.where(off_diag[g % 2] == 0, kvt_s[g], 0.0).astype(BF16) for g in range(2 * G)]

    NB = HB // 16
    DP = WC // (2 * NB)

    def relay(c):
        src = wraw.at[pl.ds(c * WC, WC)]
        dst = wqkv_s.at[pl.ds(pl.multiple_of(c * (3 * DP), 8), HB * PIT + 3 * DP)]
        for dp in range(DP):
            for nb in range(NB):
                a = _pack(src[2 * dp * NB + nb])
                b = _pack(src[(2 * dp + 1) * NB + nb])
                dst[pl.ds(8 * nb * PIT + 3 * dp, 8, stride=PIT), :] = (
                    (a & jnp.uint32(0xFFFF)) | (b << 16))
                dst[pl.ds((HP + 8 * nb) * PIT + 3 * dp, 8, stride=PIT), :] = (
                    (a >> 16) | (b & jnp.uint32(0xFFFF0000)))

    def x_tr(o):
        bx[pl.ds(o, 128), :] = bxt[:, pl.ds(o, 128)].T

    def phase2(c, carry):
        r0 = pl.multiple_of(c * T, T)
        wot_copy(c).wait()
        for i in range(NCH):
            @pl.when(c == i)
            def _():
                if i == 0:
                    bxt_copy(0).wait()
                for cc, cp in w_pieces:
                    if cc == i:
                        cp.wait()
        wq_t = wt(0, D)
        xq = _unpack(axp[:, pl.ds(r0, T)])
        pq = _dot(wq_t[:, :128], xq[:128])
        pq = _dot(wq_t[:, 128:], xq[128:]) + pq
        os_ = []
        for g in range(G):
            phis = feat(pq[g * GR:(g + 1) * GR])
            na = _dot(kvm[2 * g], phis[0])
            nb = _dot(kvm[2 * g + 1], phis[1])
            num = [na[i * 8:(i + 1) * 8] for i in range(4)] + [na[32:40] + nb[0:8]] + [
                nb[i * 8:(i + 1) * 8] for i in range(1, 5)]
            rden = pl.reciprocal(jnp.where(lo, na[40:48], nb[40:48]) + 1e-6, approx=True)
            rb = [jnp.broadcast_to(rden[j:j + 1], (8, T)) for j in range(GH)]
            for i in range(NS):
                j0, j1 = (8 * i) // DA, (8 * i + 7) // DA
                r = rb[j0] if j0 == j1 else jnp.where(sub_t < j1 * DA - 8 * i, rb[j0], rb[j1])
                os_.append(num[i] * r)
        ot = jnp.concatenate(os_, axis=0).astype(BF16)
        for hf in range(4):
            rows = slice(hf * D // 8, (hf + 1) * D // 8)
            w = _unpack(wot_a[rows, :])
            if hf == 0:
                o = _dot(w[:, :KL], ot[:KL])
                o = _dot(w[:, KL:], ot[KL:]) + o
            else:
                o = _dot(w, ot)
            aot[rows, pl.ds(r0, T)] = _pack(o.astype(BF16))
        relay(c)
        for hh in range(HC):
            h = c * HC + hh
            wo_s[pl.ds(pl.multiple_of(h * (DB // 2), DB // 2), DB // 2), :] = _pack(wot[h].T)
        x_tr(pl.multiple_of(c * 128, 128))
        return carry

    lax.fori_loop(0, NCH, phase2, 0)
    cp_mem.wait()
    for c in range(1, NCH):
        bxt_copy(c).wait()

    def wmat(i, h0=0, h1=HB, d0=0, d1=D):
        return jnp.concatenate(
            [_unpack(wqkv_s[pl.ds(((h % 2) * HP + h // 2) * PIT + 3 * ((D * i + d0) // 2),
                                  (d1 - d0) // 2, stride=3), :]) for h in range(h0, h1)], axis=1)

    scale = DB ** -0.5
    NEG = -1e9
    RA = M + SEG + M
    RB = SEG
    qi = _iota((RB, RA), 0)
    ki = _iota((RB, RA), 1)
    vis_a = (ki < M + SEG) & ((qi < M) | (qi >= ki))
    fill_a = jnp.where(ki < M + SEG, NEG, -jnp.inf).astype(F32)
    qi = _iota((RA, RA + RB), 0)
    ki = _iota((RA, RA + RB), 1)
    q_in_a = qi < M
    k_in_a = ki < M + SEG
    same = q_in_a == k_in_a
    q_mem = (qi >= 2 * M) & (qi < 3 * M)
    k_mem = (ki < M) | ((ki >= RA) & (ki < RA + M))
    q_pos = jnp.where(q_in_a, qi + (SEG - M), jnp.where(qi < 2 * M, qi - M, qi - 2 * M))
    k_pos = jnp.where(k_in_a, ki - M, jnp.where(ki < RA, ki - (M + SEG), ki - RA))
    vis_b = same & (q_mem | k_mem | (q_pos >= k_pos))
    fill_b = jnp.where(same, NEG, -jnp.inf).astype(F32)

    BT = 4 * SEG
    NIT = S // BT

    def out_copy(j):
        return pltpu.make_async_copy(out_s.at[pl.ds(j * BT, BT)], out_hbm.at[pl.ds(j * BT, BT)],
                                     osem.at[j])

    def attend(h, q_prev, k_prev, v_prev, vis, fill, first=False):
        NH = 4
        if first:
            k = _dot(h[:, KL:], wmat(0, 0, NH, KL, D))
            k = _dot(h[:, :KL], wmat(0, 0, NH, 0, KL)) + k
        else:
            k = _dot(h[:, :KL], wmat(0, 0, NH, 0, KL))
            k = _dot(h[:, KL:], wmat(0, 0, NH, KL, D)) + k
        k = jnp.concatenate([k, _dot(h, wmat(0, NH, HB))], axis=1).astype(BF16)
        q = _dot(h, wmat(1)).astype(BF16)
        if q_prev is None:
            qq, kk = q[:RB], k
        else:
            qq = jnp.concatenate([q_prev, q], axis=0)
            kk = jnp.concatenate([k_prev, k], axis=0)
        ss = [_dot_nt(qq[:, i * DB:(i + 1) * DB], kk[:, i * DB:(i + 1) * DB]) for i in range(HB)]
        v = _dot(h, wmat(2)).astype(BF16)
        vv = v if v_prev is None else jnp.concatenate([v_prev, v], axis=0)
        ps, rs = [], []
        for i in range(HB):
            sc = jnp.where(vis, ss[i] * scale, fill)
            e = jnp.exp(sc - jnp.max(sc, axis=-1, keepdims=True))
            rs.append(pl.reciprocal(jnp.sum(e, axis=-1, keepdims=True), approx=True))
            ps.append(e.astype(BF16))
        o = jnp.concatenate(
            [(_dot(ps[i], vv[:, i * DB:(i + 1) * DB]) * rs[i]).astype(BF16) for i in range(HB)],
            axis=1)
        y = _dot(o, _unpack(wo_s[...]))
        return y, q, k, v

    def pair(xx, mem, first=False):
        ha = jnp.concatenate([mem, xx[:SEG + M]], axis=0)
        ya, qa, ka, va = attend(ha, None, None, None, vis_a, fill_a, first)
        hb = jnp.concatenate([ya[:M].astype(BF16), xx[SEG + M:]], axis=0)
        yb, _, _, _ = attend(hb, qa[RB:], ka, va, vis_b, fill_b)
        yo = jnp.concatenate([ya[M:], yb[:2 * M], yb[3 * M:]], axis=0).astype(BF16)
        return yo, yb[2 * M:3 * M].astype(BF16)

    def flush(r):
        out_s[pl.ds(r, 2 * SEG), D:2 * D] = ybuf[...]

    ybuf[...] = jnp.zeros(ybuf.shape, BF16)

    def step(it, mem):
        r0 = pl.multiple_of(it * BT, BT)
        flush(pl.multiple_of(jnp.maximum(r0 - 2 * SEG, 0), 2 * SEG))
        out_s[pl.ds(r0, BT), 0:D] = _unpack(aot[:, pl.ds(r0, BT)]).T
        xx = bx[pl.ds(r0, BT), :]
        y0, mem = pair(xx[:2 * SEG], mem, True)
        out_s[pl.ds(r0, 2 * SEG), D:2 * D] = y0
        y1, mem = pair(xx[2 * SEG:], mem)
        ybuf[...] = y1
        x_tr(pl.multiple_of(jnp.minimum(r0 + NCH * BT, S - BT), BT))

        @pl.when(it > 0)
        def _():
            out_copy(it - 1).start()

        return mem

    lax.fori_loop(0, NIT, step, bmem[...])
    flush(S - 2 * SEG)
    out_copy(NIT - 1).start()
    for j in range(NIT):
        out_copy(j).wait()


@functools.partial(jax.jit, static_argnames=("seg",))
def _run(A_x, A_wqkv, A_w_phi, A_wo, B_x, B_mem0, B_Wq, B_Wk, B_Wv, B_Wo, seg):
    nb, S, D = A_x.shape
    HA, DA, _ = A_w_phi.shape
    _, HB, DB = B_Wq.shape
    M = B_mem0.shape[1]
    T = 512
    assert nb == 1 and DA == 18 and HA * DA == D and HA % 8 == 0 and D % 128 == 64
    assert DB == 128 and M == 8 and seg == 32 and S % T == 0 and HB % (2 * S // T) == 0
    nch = S // T
    kern = functools.partial(_kernel, S=S, D=D, HA=HA, DA=DA, HB=HB, DB=DB, M=M, SEG=seg, T=T)
    hbm = pl.BlockSpec(memory_space=pltpu.HBM)
    out = pl.pallas_call(
        kern,
        out_shape=jax.ShapeDtypeStruct((S, 2 * D), BF16),
        in_specs=[hbm] * 10,
        out_specs=hbm,
        scratch_shapes=[
            pltpu.VMEM((D, S), BF16),
            pltpu.VMEM((D, 3 * D), BF16),
            pltpu.VMEM((DA, DA, HA), BF16),
            pltpu.VMEM((D, D), BF16),
            pltpu.VMEM((D, S), BF16),
            pltpu.VMEM((S, D), BF16),
            pltpu.VMEM((M, D), BF16),
            pltpu.VMEM((3 * D * HB // 16, 16, DB), BF16),
            pltpu.VMEM((HB, D, DB), BF16),
            pltpu.VMEM((HB * DB // 2, D), U32),
            pltpu.VMEM(((HB + 3) * (3 * (D // 2) + 1), DB), U32),
            pltpu.VMEM((3 * D // 2, D), U32),
            pltpu.VMEM((D // 2, D), U32),
            pltpu.VMEM((D // 2, S), U32),
            pltpu.VMEM((D // 2, S), U32),
            pltpu.VMEM((HA // 4, 4 * DA, 256), U32),
            pltpu.VMEM((HA // 2, 48, 80), F32),
            pltpu.VMEM((S, 2 * D), BF16),
            pltpu.VMEM((2 * seg, D), BF16),
            pltpu.SemaphoreType.DMA((6 + 4 * nch + 2,)),
            pltpu.SemaphoreType.DMA((S // (4 * seg),)),
        ],
        compiler_params=pltpu.CompilerParams(vmem_limit_bytes=100 * 1024 * 1024),
    )(jnp.transpose(A_x[0]), A_wqkv, jnp.transpose(A_w_phi, (1, 2, 0)), A_wo,
      jnp.transpose(B_x[0]), B_mem0[0],
      B_Wq.reshape(-1, 16, DB), B_Wk.reshape(-1, 16, DB), B_Wv.reshape(-1, 16, DB),
      jnp.transpose(B_Wo, (0, 2, 1)))
    return out.reshape(1, S, 2 * D)


def pallas_concat_heads__linear_kernel_hedgehog__memory_aug_recurrent_mem_tr__prompt_kernel(
    A_x, A_wqkv, A_w_phi, A_wo, B_x, B_mem0, B_Wq, B_Wk, B_Wv, B_Wo, B_seg_len,
):
    seg = B_seg_len if isinstance(B_seg_len, int) else 32
    return _run(A_x, A_wqkv, A_w_phi, A_wo, B_x, B_mem0, B_Wq, B_Wk, B_Wv, B_Wo, seg)
```
